```python
import os as _os
_os.environ.setdefault('JAX_PLATFORMS', 'cpu')
import jax
import jax.numpy as jnp

def _softmax(x, axis=-1):
    return jax.nn.softmax(x, axis=axis)

def _gelu(x):
    return jax.nn.gelu(x, approximate=True)

def _silu(x):
    return jax.nn.silu(x)

def _sigmoid(x):
    return jax.nn.sigmoid(x)

def _layernorm(x, axis=-1, eps=1e-05):
    m = jnp.mean(x, axis=axis, keepdims=True)
    v = jnp.var(x, axis=axis, keepdims=True)
    return (x - m) / jnp.sqrt(v + eps)

def _scatter_add(tgt, idx, src, axis=0):
    return tgt.at[idx].add(src)

def _segment_sum(src, seg, n):
    return jax.ops.segment_sum(src, seg, n)

class _Rng:

    def __init__(self, key):
        self._k = key

    def _next(self):
        self._k, sub = jax.random.split(self._k)
        return sub

    def normal(self, shape):
        return jax.random.normal(self._next(), shape, dtype=jnp.bfloat16)

    def randint(self, lo, hi, shape):
        return jax.random.randint(self._next(), shape, lo, hi, dtype=jnp.int32)

    def uniform(self, shape, lo=0.0, hi=1.0):
        return jax.random.uniform(self._next(), shape, jnp.bfloat16, lo, hi)

    def permutation(self, n):
        return jax.random.permutation(self._next(), n)
kernel_name = 'adaLN_cond__ssm_conv_h3__moe_arch_mod__prompt'

def setup_inputs():
    _rng = _Rng(jax.random.key(int.from_bytes(__import__("os").urandom(4), "little")))
    _w = lambda a: (lambda t: t.astype(jnp.bfloat16) if jnp.issubdtype(t.dtype, jnp.floating) else t)(jnp.asarray(a))

    def _A_setup():
        B, S, D = (1, 2048, 640)
        ks = 4
        return {'q': _w((lambda *s: _rng.normal(s) * 0.05)(B, S, D)), 'k': _w((lambda *s: _rng.normal(s) * 0.4)(B, S, D)), 'v': _w((lambda *s: _rng.normal(s) * 0.4)(B, S, D)), 'shift_k': _w((lambda *s: _rng.normal(s) * 0.4)(D, ks) * 0.5), 'ssm_k': _w((lambda *s: _rng.normal(s) * 0.4)(D, S) * (1.0 / S ** 0.5)), 'ssm_D': _w((lambda *s: _rng.normal(s) * 0.4)(D))}
    _A_in = _A_setup()

    def _B_setup():
        B, S, D, F, C = (1, 2048, 640, 1728, 2)
        return {'x': _w((lambda *s: _rng.normal(s) * 0.05)(B, S, D)), 'w_r': _w((lambda *s: _rng.normal(s) * 0.1)(D)), 'w_gate': _w((lambda *s: _rng.normal(s) * 0.1)(D, F)), 'w_up': _w((lambda *s: _rng.normal(s) * 0.1)(D, F)), 'w_down': _w((lambda *s: _rng.normal(s) * 0.1)(F, D))}
    _B_in = _B_setup()
    return {'A_q': _A_in['q'], 'A_k': _A_in['k'], 'A_v': _A_in['v'], 'A_shift_k': _A_in['shift_k'], 'A_ssm_k': _A_in['ssm_k'], 'A_ssm_D': _A_in['ssm_D'], 'B_x': _B_in['x'], 'B_w_r': _B_in['w_r'], 'B_w_gate': _B_in['w_gate'], 'B_w_up': _B_in['w_up'], 'B_w_down': _B_in['w_down'], 'c': _w((lambda *s: _rng.normal(s) * 0.2)(1, 640) * 8.0), 'w_mod': _w((lambda *s: _rng.normal(s) * 0.2)(640, 6 * 640) * 640 ** (-0.5) * 8.0)}

def reference(A_q, A_k, A_v, A_shift_k, A_ssm_k, A_ssm_D, B_x, B_w_r, B_w_gate, B_w_up, B_w_down, c, w_mod):

    def _A_ref(q, k, v, shift_k, ssm_k, ssm_D):
        B, S, D = q.shape
        ks = shift_k.shape[-1]
        k_pad = jnp.pad(k, ((0, 0), (ks - 1, 0), (0, 0)))
        k_shift = jnp.zeros_like(k)
        for t in range(ks):
            k_shift = k_shift + k_pad[:, t:t + S, :] * shift_k[:, ks - 1 - t][None, None, :]
        kv = k_shift * v
        L = 2 * S
        kv_pad = jnp.pad(kv, ((0, 0), (0, S), (0, 0)))
        kf_pad = jnp.pad(ssm_k, ((0, 0), (0, S)))
        kv_f = (lambda x, axes=(-2, -1): jnp.fft.rfft2(x.astype(jnp.float32), axes=axes))(kv_pad[:, None, :, :], axes=(1, 2))
        kf_f = (lambda x, axes=(-2, -1): jnp.fft.rfft2(x.astype(jnp.float32), axes=axes))(kf_pad[:, None, :], axes=(1, 2))
        kf_f = (lambda x, *d: x.transpose(*d))(kf_f, 1, 2, 0)
        y_f = kv_f * kf_f[None, :, :, :]
        y = (lambda x, s, axes=(-2, -1): jnp.fft.irfft2(x, s=s, axes=axes).astype(jnp.bfloat16))(y_f, (1, L), axes=(1, 2))[:, 0, :S, :]
        y = y + kv * ssm_D[None, None, :]
        return q * y

    def _B_ref(x, w_r, w_gate, w_up, w_down):
        B, S, D = x.shape
        C = 2
        r = x @ w_r
        idx = jnp.argsort(-r, axis=-1)[:, :C]
        idx_e = jnp.repeat(idx.reshape(B, C, 1), D, axis=2)
        x_sel = jnp.take_along_axis(x, idx_e, axis=1)
        g = _silu(x_sel @ w_gate)
        u = x_sel @ w_up
        y = g * u @ w_down
        r_sel = _sigmoid(jnp.take_along_axis(r, idx, axis=1))
        y = y * r_sel.reshape(B, C, 1)
        b_off = (jnp.arange(B) * S).reshape(B, 1)
        flat_idx = (idx + b_off).reshape(B * C)
        zero = (x * 0.0).reshape(B * S, D)
        upd = _scatter_add(zero, flat_idx, y.reshape(B * C, D), axis=0)
        return x + upd.reshape(B, S, D)
    x = A_q
    mod = (_silu(c) @ w_mod).reshape(c.shape[0], 6, 1, -1)
    sa, ca, ga, sb, cb, gb = (mod[:, 0].copy(), mod[:, 1].copy(), mod[:, 2].copy(), mod[:, 3].copy(), mod[:, 4].copy(), mod[:, 5].copy())
    h = _layernorm(x, axis=-1) * (1 + ca) + sa
    x = x + ga * _A_ref(h, A_k, A_v, A_shift_k, A_ssm_k, A_ssm_D)
    h = _layernorm(x, axis=-1) * (1 + cb) + sb
    x = x + gb * _B_ref(h, B_w_r, B_w_gate, B_w_up, B_w_down)
    return x
```

```python
import math
import numpy as np
import jax
import jax.numpy as jnp
from jax import lax
import jax.experimental.pallas as pl
import jax.experimental.pallas.tpu as pltpu

S = 2048
D = 640
FF = 1728
B = 128
NB = S // B
NT = D // 128
NG = B // 8
EPS = 1e-5
KV_CH = 256
NKV = S // KV_CH
Q_CH = 256
NQ = S // Q_CH
GPI = 4
F_CHUNKS = ((0, 512), (512, 512), (1024, 512), (1536, 192))
BIG = 1 << 20
SCOPES = False

f32 = jnp.float32
bf16 = jnp.bfloat16
u32 = jnp.uint32


def _dft_consts():
    k = np.concatenate([np.arange(0, B, 2), np.arange(1, B, 2)]).astype(np.float64)
    n = np.arange(B, dtype=np.float64)
    th = 2.0 * np.pi * (k[:, None] + 0.5) * n[None, :] / (2 * B)
    fwd = np.stack([np.cos(th).reshape(NG, 8, B), -np.sin(th).reshape(NG, 8, B)], axis=1).reshape(2 * B, B)
    n2 = np.arange(B, 2 * B, dtype=np.float64)
    th2 = 2.0 * np.pi * (k[None, :] + 0.5) * n2[:, None] / (2 * B)
    inv = np.stack([np.cos(th2).reshape(B, NG, 8), -np.sin(th2).reshape(B, NG, 8)], axis=2).reshape(B, 2 * B) / B
    inv = np.concatenate([inv[:, :B], inv[:, B:]], axis=0)
    return np.concatenate([fwd, inv], axis=0).astype(np.float32)


class _Scope:
    def __init__(self, name):
        self.cm = jax.named_scope(name) if SCOPES else None

    def __enter__(self):
        if self.cm is not None:
            self.cm.__enter__()

    def __exit__(self, *a):
        if self.cm is not None:
            self.cm.__exit__(*a)


def _rsqrt(v):
    return jnp.exp2(jnp.log(v) * (-0.5 / math.log(2.0)))


def _kernel(q_hbm, k_hbm, v_hbm, sk_hbm, h_hbm, dd_hbm, wr_hbm, wg_hbm, wu_hbm, wd_hbm,
            c_hbm, wm_hbm, fc_hbm,
            out_hbm,
            q_buf, k_buf, v_buf, sk_buf, h_buf, dd_buf, wr_buf, wg_buf, wu_buf, wd_buf,
            c_buf, wm_buf, fc_buf,
            k32, prev, u_s, g_a, g_b, y_a, y_b, y_lo, y_hi, xc_s, x2_s, xc2_s,
            st1, st2, st3, st4, st5, o_buf, par, r_s, zs,
            sem, sem_o):
    o_small, o_h, o_k, o_v, o_wm, o_q, o_w = [int(o) for o in np.cumsum([0, 5, NT, NKV, NKV, 1, NQ])]
    small = [(fc_hbm, fc_buf), (sk_hbm, sk_buf), (dd_hbm, dd_buf), (c_hbm, c_buf), (wr_hbm, wr_buf)]
    cp_small = [pltpu.make_async_copy(s, d, sem.at[o_small + i]) for i, (s, d) in enumerate(small)]

    def cp_h(j, m):
        return pltpu.make_async_copy(h_hbm.at[pl.ds(j * 128, 128), pl.ds(m * B, B)], h_buf.at[j, m], sem.at[o_h + j])

    def cp_rows(src, dst, off, i, rows):
        return pltpu.make_async_copy(src.at[pl.ds(i * rows, rows)], dst.at[pl.ds(i * rows, rows)], sem.at[off + i])

    cp_wm = pltpu.make_async_copy(wm_hbm, wm_buf, sem.at[o_wm])

    def cp_w(ci, t):
        f0, fn = F_CHUNKS[ci]
        src, dst = ((wg_hbm, wg_buf), (wu_hbm, wu_buf), (wd_hbm, wd_buf))[t]
        return pltpu.make_async_copy(src.at[pl.ds(f0, fn)], dst.at[pl.ds(f0, fn)], sem.at[o_w + ci * 3 + t])

    cp_small[0].start()
    for m in range(NB):
        cp_h(0, m).start()
    for c in cp_small[1:]:
        c.start()
    for i in range(NKV):
        cp_rows(k_hbm, k_buf, o_k, i, KV_CH).start()
        cp_rows(v_hbm, v_buf, o_v, i, KV_CH).start()
    def start_h(j):
        for m in range(NB):
            cp_h(j, m).start()

    start_h(1)

    for t in range(4):
        zs[t] = 0
    for j in range(NT):
        k32[j, 0:8, :] = jnp.zeros((8, 128), f32)
        prev[j] = jnp.zeros((NG, 2, 8, 128), f32)

    nt_dims = (((1,), (1,)), ((), ()))
    fc_w = fc_buf.bitcast(u32)
    h_w = h_buf.bitcast(u32)
    ya_w = y_a.bitcast(u32)
    yb_w = y_b.bitcast(u32)

    def as_bf16(w):
        return pltpu.bitcast(w, bf16)

    def f_fwd():
        return as_bf16(fc_w[0:B, :])

    def wait_h(j):
        for m in range(NB):
            cp_h(j, m).wait()

    def stage_h(j, m, g_dst):
        hh = lax.dot_general(f_fwd(), as_bf16(h_w[j, m]), nt_dims, preferred_element_type=f32)
        g_dst[m] = hh.reshape(NG, 2, 8, 128)

    def fix_d(j, g_dst):
        dj = dd_buf[j:j + 1, :].astype(f32)[None]
        g_dst[0, :, 0] = g_dst[0, :, 0] + dj

    def stage_i(j, a, y_src_w):
        rows = pl.ds(pl.multiple_of(a * B, B), B)
        hb = B // 2
        y_lo[j, rows, :] = jnp.dot(as_bf16(fc_w[B:B + hb, :]), as_bf16(y_src_w[a, 0:hb]), preferred_element_type=f32)
        y_hi[j, rows, :] = jnp.dot(as_bf16(fc_w[B + hb:, :]), as_bf16(y_src_w[a, hb:]), preferred_element_type=f32)

    def stage_c(j, g, g_src, y_dst):
        for half in range(2):
            gg = g + zs[half]
            g2 = g + zs[2 + half]
            lo = half * 8
            n_in = lo + 8
            res = []
            for comp in range(3):
                acc = [None] * 8 if comp == 0 else list(res[0])
                v = {}
                for jj in range(n_in):
                    u = u_s[j, jj, comp, gg]
                    for o in range(8):
                        m = lo + o - jj
                        if m < 0:
                            continue
                        if m not in v:
                            if comp == 0:
                                v[m] = g_src[m, g2, 0] + g_src[m, g2, 1]
                            else:
                                v[m] = g_src[m, gg, comp - 1]
                        p = u * v[m]
                        if acc[o] is None:
                            acc[o] = p
                        elif comp == 2:
                            acc[o] = acc[o] - p
                        else:
                            acc[o] = acc[o] + p
                res.append(acc)
            for o in range(8):
                y_dst[lo + o, pl.ds(pl.multiple_of(g * 16, 16), 16), :] = (
                    jnp.concatenate([res[2][o], res[1][o]], axis=0).astype(bf16))

    inv_d = 1.0 / D

    def lanes(t):
        return slice(t * 128, (t + 1) * 128)

    def rsum(xs):
        s = xs[0]
        for x in xs[1:]:
            s = s + x
        return jnp.broadcast_to(jnp.sum(s, axis=1, keepdims=True), (8, 128))

    def grp(r0, gi):
        return pl.ds(pl.multiple_of(r0 + gi * 8, 8), 8)

    def stage_a(r0, nrows):
        for gi in range(nrows // 8):
            rows = grp(r0, gi)
            st1[rows, :] = rsum([q_buf[rows, lanes(t)].astype(f32) for t in range(NT)])

    def stage_b(r0, nrows):
        for gi in range(nrows // 8):
            rows = grp(r0, gi)
            mu = st1[rows, :] * inv_d
            sq = []
            for t in range(NT):
                xc = q_buf[rows, lanes(t)].astype(f32) - mu
                xc_s[t, rows, :] = xc
                sq.append(xc * xc)
            st2[rows, :] = rsum(sq)

    def stage_x(r0):
        for gi in range(NG):
            rows = grp(r0, gi)
            rs = _rsqrt(st2[rows, :] * inv_d + EPS)
            xs = []
            for t in range(NT):
                xc = xc_s[t, rows, :]
                y = y_lo[t, rows, :] + y_hi[t, rows, :]
                x2 = ((xc * rs) * par[0, :, lanes(t)] + par[1, :, lanes(t)]) * y + xc
                x2_s[t, rows, :] = x2
                xs.append(x2)
            st3[rows, :] = rsum(xs)

    def stage_d(r0):
        for gi in range(NG):
            rows = grp(r0, gi)
            mu = st3[rows, :] * inv_d
            sq, rd = [], []
            for t in range(NT):
                xc = x2_s[t, rows, :] - mu
                xc2_s[t, rows, :] = xc
                sq.append(xc * xc)
                rd.append(xc * par[4, :, lanes(t)])
            st4[rows, :] = rsum(sq)
            st5[rows, :] = rsum(rd)

    lane = lax.broadcasted_iota(jnp.int32, (8, 128), 1)

    def stage_e(a, r0):
        rblk = jnp.full((8, 128), -jnp.inf, f32)
        for gi in range(NG):
            rows = grp(r0, gi)
            rs = _rsqrt(st4[rows, :] * inv_d + EPS)
            mu = (st1[rows, :] + st3[rows, :]) * inv_d
            rblk = jnp.where(lane == gi, st5[rows, :] * rs, rblk)
            for t in range(NT):
                xc = xc2_s[t, rows, :]
                out = (xc * rs) * par[2, :, lanes(t)] + xc + (par[3, :, lanes(t)] + mu)
                o_buf[rows, lanes(t)] = out.astype(bf16)
        r_s[a] = rblk

    cp_small[0].wait()
    wait_h(0)

    def h0_body(i, c):
        for t in range(4):
            stage_h(0, i * 4 + t, g_a)
        return c
    with _Scope('ph0'):
        lax.fori_loop(0, NB // 4, h0_body, 0)
    start_h(2)
    start_h(3)
    for c in cp_small[1:]:
        c.wait()
    fix_d(0, g_a)

    def p_body(i, c):
        cp_rows(k_hbm, k_buf, o_k, i, KV_CH).wait()
        cp_rows(v_hbm, v_buf, o_v, i, KV_CH).wait()
        sk = sk_buf[...].astype(f32)
        nblk = KV_CH // B
        for j in range(NT):
            ls = lanes(j)
            for t in range(nblk):
                a = i * nblk + t
                r0 = pl.multiple_of(a * B, B)
                kf = k_buf[pl.ds(r0, B), ls].astype(f32)
                k32[j, pl.ds(r0 + 8, B), :] = kf
                ks = kf * sk[0:1, ls]
                for t2 in range(1, 4):
                    ks = ks + k32[j, pl.ds(r0 + 8 - t2, B), :] * sk[t2:t2 + 1, ls]
                kv = (ks * v_buf[pl.ds(r0, B), ls].astype(f32)).astype(bf16)
                x = jnp.dot(f_fwd(), kv, preferred_element_type=f32).reshape(NG, 2, 8, 128)
                p = prev[j] if t == 0 else xprev
                xprev = x
                if t == nblk - 1:
                    prev[j] = x
                hb = NG // 2
                wr_ = jnp.concatenate([p[:hb, 0] + x[:hb, 1], p[hb:, 0] - x[hb:, 1]], axis=0)
                wi_ = jnp.concatenate([p[:hb, 1] - x[:hb, 0], p[hb:, 1] + x[hb:, 0]], axis=0)
                u_s[j, a, 0] = wr_
                u_s[j, a, 1] = wi_ - wr_
                u_s[j, a, 2] = wr_ + wi_
        return c
    with _Scope('ph1'):
        lax.fori_loop(0, NKV, p_body, 0)

    start_h(4)
    cp_wm.start()
    for i in range(NQ):
        cp_rows(q_hbm, q_buf, o_q, i, Q_CH).start()
    gs = (g_a, g_b)
    ys = (y_a, y_b)
    ysw = (ya_w, yb_w)
    n_it = NG // GPI
    rows_it = S // n_it
    for j in range(NT):
        if j + 1 < NT:
            wait_h(j + 1)
        else:
            with _Scope('mod'):
                cp_wm.wait()
                cf = c_buf[...].astype(f32)
                cs = (cf * jax.nn.sigmoid(cf)).astype(bf16)
                mod = jnp.dot(jnp.broadcast_to(cs, (16, D)), wm_buf[...], preferred_element_type=f32)[0:8]
                sa, ca, ga, sb, cb, gb = [mod[:, i * D:(i + 1) * D] for i in range(6)]
                wr = jnp.concatenate([jnp.broadcast_to(wr_buf[t:t + 1, :].astype(f32), (8, 128))
                                      for t in range(NT)], axis=1)
                par[0] = ga * (1.0 + ca)
                par[1] = ga * sa
                par[2] = gb * (1.0 + cb)
                par[3] = gb * sb
                par[4] = (1.0 + cb) * wr
                par[5] = wr
                par[6] = 1.0 + cb
                par[7] = sb
                par[8] = gb

        def c_body(i, c, j=j):
            if j == NT - 1:
                for t in range(rows_it // Q_CH):
                    cp_rows(q_hbm, q_buf, o_q, i * (rows_it // Q_CH) + t, Q_CH).wait()
                stage_a(i * rows_it, rows_it)
            for t in range(GPI):
                g = i * GPI + t
                if j + 1 < NT:
                    stage_h(j + 1, g, gs[(j + 1) % 2])
                if j > 0:
                    stage_i(j - 1, g, ysw[(j - 1) % 2])
                stage_c(j, g, gs[j % 2], ys[j % 2])
            return c
        with _Scope('ph2_%d' % j):
            lax.fori_loop(0, n_it, c_body, 0)
        if j == 0:
            for ci in range(len(F_CHUNKS)):
                for t in range(3):
                    cp_w(ci, t).start()
        if j + 1 < NT:
            fix_d(j + 1, gs[(j + 1) % 2])

    def ib_body(i, c):
        for t in range(4):
            stage_i(NT - 1, i * 4 + t, ysw[(NT - 1) % 2])
        stage_b(i * 4 * B, 4 * B)
        return c
    with _Scope('ph3_ib'):
        lax.fori_loop(0, NB // 4, ib_body, 0)

    with _Scope('ph3_pro'):
        stage_x(0)
        stage_x(B)
        stage_d(0)

    def e_body(a, c):
        stage_x((a + 2) * B)
        stage_d((a + 1) * B)
        stage_e(a, a * B)
        return c
    with _Scope('ph3'):
        lax.fori_loop(0, NB - 2, e_body, 0)
    with _Scope('ph3_epi'):
        stage_d((NB - 1) * B)
        stage_e(NB - 2, (NB - 2) * B)
        stage_e(NB - 1, (NB - 1) * B)

    rall = r_s[...]
    sh = (NB, 8, 128)
    l3 = lax.broadcasted_iota(jnp.int32, sh, 2)
    ridx = (lax.broadcasted_iota(jnp.int32, sh, 0) * B + l3 * 8
            + lax.broadcasted_iota(jnp.int32, sh, 1))
    ridx = jnp.where(l3 < NG, ridx, BIG)
    m1 = jnp.max(rall)
    i1 = jnp.min(jnp.where(rall == m1, ridx, BIG))
    rall2 = jnp.where(ridx == i1, -jnp.inf, rall)
    m2 = jnp.max(rall2)
    i2 = jnp.min(jnp.where(jnp.logical_and(rall2 == m2, ridx != i1), ridx, BIG))
    i1 = jnp.clip(i1, 0, S - 1)
    i2 = jnp.clip(i2, 0, S - 1)

    row16 = lax.broadcasted_iota(jnp.int32, (16, 128), 0)

    def pick(ref_rows):
        return jnp.where(row16 == 0, ref_rows(i1), jnp.where(row16 == 1, ref_rows(i2), 0.0))

    xc = jnp.concatenate([pick(lambda i, t=t: xc2_s[t, pl.ds(i, 1), :]) for t in range(NT)], axis=1)
    rs = _rsqrt(pick(lambda i: st4[pl.ds(i, 1), :]) * inv_d + EPS)[:, 0:1]
    mu = (pick(lambda i: st1[pl.ds(i, 1), :] + st3[pl.ds(i, 1), :]) * inv_d)[:, 0:1]
    h2 = xc * rs * par[6, 0:1] + par[7, 0:1]
    gate = jax.nn.sigmoid(jnp.sum(h2 * par[5, 0:1], axis=1, keepdims=True))
    h2b = h2.astype(bf16)

    c1 = i1 // B
    c2 = i2 // B
    c2 = jnp.where(c1 == c2, (c1 + 1) % NB, c2)
    lo = jnp.minimum(c1, c2)
    hi = jnp.maximum(c1, c2)

    def cp_out(blk, s):
        r = pl.ds(pl.multiple_of(blk * B, B), B)
        return pltpu.make_async_copy(o_buf.at[r], out_hbm.at[r], sem_o.at[s])

    def early_blk(s):
        o = s + (s >= lo).astype(jnp.int32)
        return o + (o >= hi).astype(jnp.int32)

    acc = jnp.zeros((16, D), f32)
    with _Scope('mlp'):
        for ci, (f0, fn) in enumerate(F_CHUNKS):
            if ci == 0:
                for c2_ in range(len(F_CHUNKS) - 1):
                    for t in range(3):
                        cp_w(c2_, t).wait()
                for s in range(NB - 2):
                    cp_out(early_blk(s), s).start()
            if ci == len(F_CHUNKS) - 1:
                for t in range(3):
                    cp_w(ci, t).wait()
            gg = lax.dot_general(h2b, wg_buf[f0:f0 + fn, :], nt_dims, preferred_element_type=f32)
            uu = lax.dot_general(h2b, wu_buf[f0:f0 + fn, :], nt_dims, preferred_element_type=f32)
            act = (gg * jax.nn.sigmoid(gg) * uu).astype(bf16)
            acc = acc + jnp.dot(act, wd_buf[f0:f0 + fn, :], preferred_element_type=f32)
    o_sel = xc + mu + par[8, 0:1] * (h2 + acc * gate)

    row16d = lax.broadcasted_iota(jnp.int32, (16, D), 0)
    for t, idx in enumerate((i1, i2)):
        base = pl.multiple_of((idx // 16) * 16, 16)
        tile = o_buf[pl.ds(base, 16), :].astype(f32)
        tile = jnp.where(row16d == idx - base, o_sel[t:t + 1], tile)
        o_buf[pl.ds(base, 16), :] = tile.astype(bf16)
    cp_out(lo, NB - 2).start()
    cp_out(hi, NB - 1).start()
    for s in range(NB - 2):
        cp_out(early_blk(s), s).wait()
    cp_out(lo, NB - 2).wait()
    cp_out(hi, NB - 1).wait()


@jax.jit
def pallas_adaLN_cond__ssm_conv_h3__moe_arch_mod__prompt_kernel(
    A_q, A_k, A_v, A_shift_k, A_ssm_k, A_ssm_D, B_x, B_w_r, B_w_gate, B_w_up, B_w_down, c, w_mod,
):
    del B_x
    args = (
        A_q.reshape(S, D), A_k.reshape(S, D), A_v.reshape(S, D), A_shift_k.T, A_ssm_k,
        A_ssm_D.reshape(NT, 128), B_w_r.reshape(NT, 128), B_w_gate.T, B_w_up.T, B_w_down,
        c, w_mod, jnp.asarray(_dft_consts(), bf16),
    )
    vm = pltpu.VMEM
    in_bufs = [vm(a.shape, a.dtype) for a in args]
    in_bufs[4] = vm((NT, NB, 128, B), bf16)
    scratch = in_bufs + [
        vm((NT, S + 8, 128), f32),
        vm((NT, NG, 2, 8, 128), f32),
        vm((NT, NB, 3, NG, 8, 128), f32),
        vm((NB, NG, 2, 8, 128), f32),
        vm((NB, NG, 2, 8, 128), f32),
        vm((NB, 2 * B, 128), bf16),
        vm((NB, 2 * B, 128), bf16),
        vm((NT, S, 128), f32),
        vm((NT, S, 128), f32),
        vm((NT, S, 128), f32),
        vm((NT, S, 128), f32),
        vm((NT, S, 128), f32),
        vm((S, 128), f32),
        vm((S, 128), f32),
        vm((S, 128), f32),
        vm((S, 128), f32),
        vm((S, 128), f32),
        vm((S, D), bf16),
        vm((9, 8, D), f32),
        vm((NB, 8, 128), f32),
        pltpu.SMEM((4,), jnp.int32),
        pltpu.SemaphoreType.DMA((5 + NT + 2 * NKV + 1 + NQ + 3 * len(F_CHUNKS),)),
        pltpu.SemaphoreType.DMA((NB,)),
    ]
    out = pl.pallas_call(
        _kernel,
        out_shape=jax.ShapeDtypeStruct((S, D), bf16),
        in_specs=[pl.BlockSpec(memory_space=pl.ANY)] * len(args),
        out_specs=pl.BlockSpec(memory_space=pl.ANY),
        scratch_shapes=scratch,
        compiler_params=pltpu.CompilerParams(vmem_limit_bytes=120 * 1024 * 1024),
        name="adaln_h3_mod",
    )(*args)
    return out.reshape(1, S, D)
```

```python
import math
import numpy as np
import jax
import jax.numpy as jnp
from jax import lax
import jax.experimental.pallas as pl
import jax.experimental.pallas.tpu as pltpu

S = 2048
D = 640
FF = 1728
B = 128
NB = S // B
NT = D // 128
NG = B // 8
EPS = 1e-5
KV_CH = 256
NKV = S // KV_CH
Q_CH = 256
NQ = S // Q_CH
GPI = 4
F_CHUNKS = ((0, 512), (512, 512), (1024, 512), (1536, 192))
BIG = 1 << 20
SCOPES = False

f32 = jnp.float32
bf16 = jnp.bfloat16
u32 = jnp.uint32


def _dft_consts():
    k = np.concatenate([np.arange(0, B, 2), np.arange(1, B, 2)]).astype(np.float64)
    n = np.arange(B, dtype=np.float64)
    th = 2.0 * np.pi * (k[:, None] + 0.5) * n[None, :] / (2 * B)
    fwd = np.stack([np.cos(th).reshape(NG, 8, B), -np.sin(th).reshape(NG, 8, B)], axis=1).reshape(2 * B, B)
    n2 = np.arange(B, 2 * B, dtype=np.float64)
    th2 = 2.0 * np.pi * (k[None, :] + 0.5) * n2[:, None] / (2 * B)
    inv = np.stack([np.cos(th2).reshape(B, NG, 8), -np.sin(th2).reshape(B, NG, 8)], axis=2).reshape(B, 2 * B) / B
    inv = np.concatenate([inv[:, :B], inv[:, B:]], axis=0)
    return np.concatenate([fwd, inv], axis=0).astype(np.float32)


class _Scope:
    def __init__(self, name):
        self.cm = jax.named_scope(name) if SCOPES else None

    def __enter__(self):
        if self.cm is not None:
            self.cm.__enter__()

    def __exit__(self, *a):
        if self.cm is not None:
            self.cm.__exit__(*a)


def _rs(ssq):
    return jnp.exp2(jnp.log(ssq + D * EPS) * (-0.5 / math.log(2.0)))


def _body(q_hbm, k_hbm, v_hbm, sk_hbm, h_hbm, dd_hbm, wr_hbm, wg_hbm, wu_hbm, wd_hbm,
            c_hbm, wm_hbm, fc_hbm,
            out_hbm,
            q_buf, k_buf, v_buf, sk_buf, h_buf, dd_buf, wr_buf, wg_buf, wu_buf, wd_buf,
            c_buf, wm_buf, fc_buf,
            k32, prev, u_s, g_a, g_b, y_a, y_b, y_lo, y_hi, xc_s, x2_s, xc2_s,
            st1, st2, st3, st4, st5, o_buf, par, r_s, zs,
            sem_o, sem):
    o_small, o_h, o_k, o_v, o_wm, o_q, o_w = [int(o) for o in np.cumsum([0, 5, NT, NKV, NKV, 1, NQ])]
    small = [(fc_hbm, fc_buf), (sk_hbm, sk_buf), (dd_hbm, dd_buf), (c_hbm, c_buf), (wr_hbm, wr_buf)]
    cp_small = [pltpu.make_async_copy(s, d, sem.at[o_small + i]) for i, (s, d) in enumerate(small)]

    def cp_h(j, m):
        return pltpu.make_async_copy(h_hbm.at[pl.ds(j * 128, 128), pl.ds(m * B, B)], h_buf.at[j, m], sem.at[o_h + j])

    def cp_rows(src, dst, off, i, rows):
        return pltpu.make_async_copy(src.at[pl.ds(i * rows, rows)], dst.at[pl.ds(i * rows, rows)], sem.at[off + i])

    cp_wm = pltpu.make_async_copy(wm_hbm, wm_buf, sem.at[o_wm])

    def cp_w(ci, t):
        f0, fn = F_CHUNKS[ci]
        src, dst = ((wg_hbm, wg_buf), (wu_hbm, wu_buf), (wd_hbm, wd_buf))[t]
        return pltpu.make_async_copy(src.at[pl.ds(f0, fn)], dst.at[pl.ds(f0, fn)], sem.at[o_w + ci * 3 + t])

    cp_small[0].start()
    for m in range(NB):
        cp_h(0, m).start()
    for c in cp_small[1:]:
        c.start()
    for i in range(NKV):
        cp_rows(k_hbm, k_buf, o_k, i, KV_CH).start()
        cp_rows(v_hbm, v_buf, o_v, i, KV_CH).start()
    def start_h(j):
        for m in range(NB):
            cp_h(j, m).start()

    start_h(1)

    for t in range(4):
        zs[t] = 0
    for j in range(NT):
        k32[j, 0:8, :] = jnp.zeros((8, 128), f32)
        prev[j] = jnp.zeros((NG, 2, 8, 128), f32)
    r_s[...] = jnp.zeros((2, 8, 128), f32)

    nt_dims = (((1,), (1,)), ((), ()))
    fc_w = fc_buf.bitcast(u32)
    h_w = h_buf.bitcast(u32)
    ya_w = y_a.bitcast(u32)
    yb_w = y_b.bitcast(u32)

    def as_bf16(w):
        return pltpu.bitcast(w, bf16)

    def f_fwd():
        return as_bf16(fc_w[0:B, :])

    def wait_h(j):
        for m in range(NB):
            cp_h(j, m).wait()

    def stage_h(j, m, g_dst):
        hh = lax.dot_general(f_fwd(), as_bf16(h_w[j, m]), nt_dims, preferred_element_type=f32)
        g_dst[m] = hh.reshape(NG, 2, 8, 128)

    def fix_d(j, g_dst):
        dj = dd_buf[j:j + 1, :].astype(f32)[None]
        g_dst[0, :, 0] = g_dst[0, :, 0] + dj

    def stage_i(j, a, y_src_w):
        rows = pl.ds(pl.multiple_of(a * B, B), B)
        hb = B // 2
        y_lo[j, rows, :] = jnp.dot(as_bf16(fc_w[B:B + hb, :]), as_bf16(y_src_w[a, 0:hb]), preferred_element_type=f32)
        y_hi[j, rows, :] = jnp.dot(as_bf16(fc_w[B + hb:, :]), as_bf16(y_src_w[a, hb:]), preferred_element_type=f32)

    def stage_c(j, g, g_src, y_dst):
        for half in range(2):
            gg = g + zs[half]
            g2 = g + zs[2 + half]
            lo = half * 8
            n_in = lo + 8
            res = []
            for comp in range(3):
                acc = [None] * 8 if comp == 0 else list(res[0])
                v = {}
                for jj in range(n_in):
                    u = u_s[j, jj, comp, gg]
                    for o in range(8):
                        m = lo + o - jj
                        if m < 0:
                            continue
                        if m not in v:
                            if comp == 0:
                                v[m] = g_src[m, g2, 0] + g_src[m, g2, 1]
                            else:
                                v[m] = g_src[m, gg, comp - 1]
                        p = u * v[m]
                        if acc[o] is None:
                            acc[o] = p
                        elif comp == 2:
                            acc[o] = acc[o] - p
                        else:
                            acc[o] = acc[o] + p
                res.append(acc)
            for o in range(8):
                y_dst[lo + o, pl.ds(pl.multiple_of(g * 16, 16), 16), :] = (
                    jnp.concatenate([res[2][o], res[1][o]], axis=0).astype(bf16))

    inv_d = 1.0 / D

    def lanes(t):
        return slice(t * 128, (t + 1) * 128)

    def rsum(xs):
        s = xs[0]
        for x in xs[1:]:
            s = s + x
        return jnp.broadcast_to(jnp.sum(s, axis=1, keepdims=True), (8, 128))

    def grp(r0, gi):
        return pl.ds(pl.multiple_of(r0 + gi * 8, 8), 8)

    def stage_a(r0, nrows):
        for gi in range(nrows // 8):
            rows = grp(r0, gi)
            st1[rows, :] = rsum([q_buf[rows, lanes(t)].astype(f32) for t in range(NT)]) * inv_d

    def stage_b(r0, nrows):
        for gi in range(nrows // 8):
            rows = grp(r0, gi)
            mu = st1[rows, :]
            sq = []
            for t in range(NT):
                xc = q_buf[rows, lanes(t)].astype(f32) - mu
                xc_s[t, rows, :] = xc
                sq.append(xc * xc)
            st2[rows, :] = _rs(rsum(sq))

    def stage_x(r0):
        for gi in range(NG):
            rows = grp(r0, gi)
            rs = st2[rows, :]
            xs = []
            for t in range(NT):
                xc = xc_s[t, rows, :]
                y = y_lo[t, rows, :] + y_hi[t, rows, :]
                x2 = ((xc * rs) * par[0, :, lanes(t)] + par[1, :, lanes(t)]) * y + xc
                x2_s[t, rows, :] = x2
                xs.append(x2)
            st3[rows, :] = rsum(xs) * inv_d

    def stage_d(r0):
        for gi in range(NG):
            rows = grp(r0, gi)
            mu = st3[rows, :]
            sq, rd = [], []
            for t in range(NT):
                xc = x2_s[t, rows, :] - mu
                xc2_s[t, rows, :] = xc
                sq.append(xc * xc)
                rd.append(xc * par[4, :, lanes(t)])
            rs = _rs(rsum(sq))
            st4[rows, :] = rs
            st5[rows, :] = rsum(rd) * rs

    lane = lax.broadcasted_iota(jnp.int32, (8, 128), 1)

    def stage_e(a, r0):
        rblk = r_s[a // 8]
        lane_rel = lane - (a % 8) * NG
        for gi in range(NG):
            rows = grp(r0, gi)
            rs = st4[rows, :]
            mu = st1[rows, :] + st3[rows, :]
            rblk = jnp.where(lane_rel == gi, st5[rows, :], rblk)
            for t in range(NT):
                xc = xc2_s[t, rows, :]
                out = (xc * rs) * par[2, :, lanes(t)] + xc + (par[3, :, lanes(t)] + mu)
                o_buf[rows, lanes(t)] = out.astype(bf16)
        r_s[a // 8] = rblk

    cp_small[0].wait()
    wait_h(0)

    def h0_body(i, c):
        for t in range(4):
            stage_h(0, i * 4 + t, g_a)
        return c
    with _Scope('ph0'):
        lax.fori_loop(0, NB // 4, h0_body, 0)
    start_h(2)
    start_h(3)
    for c in cp_small[1:]:
        c.wait()
    fix_d(0, g_a)

    def p_body(i, c):
        cp_rows(k_hbm, k_buf, o_k, i, KV_CH).wait()
        cp_rows(v_hbm, v_buf, o_v, i, KV_CH).wait()
        sk = sk_buf[...].astype(f32)
        nblk = KV_CH // B
        for j in range(NT):
            ls = lanes(j)
            for t in range(nblk):
                a = i * nblk + t
                r0 = pl.multiple_of(a * B, B)
                kf = k_buf[pl.ds(r0, B), ls].astype(f32)
                k32[j, pl.ds(r0 + 8, B), :] = kf
                ks = kf * sk[0:1, ls]
                for t2 in range(1, 4):
                    ks = ks + k32[j, pl.ds(r0 + 8 - t2, B), :] * sk[t2:t2 + 1, ls]
                kv = (ks * v_buf[pl.ds(r0, B), ls].astype(f32)).astype(bf16)
                x = jnp.dot(f_fwd(), kv, preferred_element_type=f32).reshape(NG, 2, 8, 128)
                p = prev[j] if t == 0 else xprev
                xprev = x
                if t == nblk - 1:
                    prev[j] = x
                hb = NG // 2
                wr_ = jnp.concatenate([p[:hb, 0] + x[:hb, 1], p[hb:, 0] - x[hb:, 1]], axis=0)
                wi_ = jnp.concatenate([p[:hb, 1] - x[:hb, 0], p[hb:, 1] + x[hb:, 0]], axis=0)
                u_s[j, a, 0] = wr_
                u_s[j, a, 1] = wi_ - wr_
                u_s[j, a, 2] = wr_ + wi_
        return c
    with _Scope('ph1'):
        lax.fori_loop(0, NKV, p_body, 0)

    start_h(4)
    cp_wm.start()
    for i in range(NQ):
        cp_rows(q_hbm, q_buf, o_q, i, Q_CH).start()
    gs = (g_a, g_b)
    ys = (y_a, y_b)
    ysw = (ya_w, yb_w)
    n_it = NG // GPI
    rows_it = S // n_it
    for j in range(NT):
        if j + 1 < NT:
            wait_h(j + 1)
        else:
            with _Scope('mod'):
                cp_wm.wait()
                cf = c_buf[...].astype(f32)
                cs = (cf * jax.nn.sigmoid(cf)).astype(bf16)
                mod = jnp.dot(jnp.broadcast_to(cs, (16, D)), wm_buf[...], preferred_element_type=f32)[0:8]
                sa, ca, ga, sb, cb, gb = [mod[:, i * D:(i + 1) * D] for i in range(6)]
                wr = jnp.concatenate([jnp.broadcast_to(wr_buf[t:t + 1, :].astype(f32), (8, 128))
                                      for t in range(NT)], axis=1)
                sqd = math.sqrt(D)
                par[0] = ga * (1.0 + ca) * sqd
                par[1] = ga * sa
                par[2] = gb * (1.0 + cb) * sqd
                par[3] = gb * sb
                par[4] = (1.0 + cb) * wr
                par[5] = wr
                par[6] = (1.0 + cb) * sqd
                par[7] = sb
                par[8] = gb

        def c_body(i, c, j=j):
            if j == NT - 1:
                for t in range(rows_it // Q_CH):
                    cp_rows(q_hbm, q_buf, o_q, i * (rows_it // Q_CH) + t, Q_CH).wait()
                stage_a(i * rows_it, rows_it)
                if i > 0:
                    stage_b((i - 1) * rows_it, rows_it)
            for t in range(GPI):
                g = i * GPI + t
                if j + 1 < NT:
                    stage_h(j + 1, g, gs[(j + 1) % 2])
                if j > 0:
                    stage_i(j - 1, g, ysw[(j - 1) % 2])
                stage_c(j, g, gs[j % 2], ys[j % 2])
            return c
        with _Scope('ph2_%d' % j):
            if j == NT - 1:
                for i in range(n_it):
                    c_body(i, 0)
            else:
                lax.fori_loop(0, n_it, c_body, 0)
        if j == 0:
            for ci in range(len(F_CHUNKS)):
                for t in range(3):
                    cp_w(ci, t).start()
        if j + 1 < NT:
            fix_d(j + 1, gs[(j + 1) % 2])

    y_last = ysw[(NT - 1) % 2]
    with _Scope('ph3_pro'):
        for a in range(3):
            stage_i(NT - 1, a, y_last)
        stage_b(S - rows_it, rows_it)
        stage_x(0)
        stage_x(B)
        stage_d(0)

    def e_body(a, c):
        stage_i(NT - 1, a + 3, y_last)
        stage_x((a + 2) * B)
        stage_d((a + 1) * B)
        stage_e(a, a * B)
        return c
    with _Scope('ph3'):
        lax.fori_loop(0, NB - 3, e_body, 0)
    with _Scope('ph3_epi'):
        stage_x((NB - 1) * B)
        stage_d((NB - 2) * B)
        stage_e(NB - 3, (NB - 3) * B)
        stage_d((NB - 1) * B)
        stage_e(NB - 2, (NB - 2) * B)
        stage_e(NB - 1, (NB - 1) * B)

    rall = r_s[...].reshape(16, 128)
    sub = lax.broadcasted_iota(jnp.int32, (16, 128), 0)
    ln = lax.broadcasted_iota(jnp.int32, (16, 128), 1)
    ridx = (sub // 8) * (S // 2) + ln * 8 + (sub % 8)
    kbits = (lax.bitcast_convert_type(rall, jnp.int32) & jnp.int32(-2048)) | (S - 1 - ridx)
    key = lax.bitcast_convert_type(kbits, f32)
    m1 = jnp.max(key, axis=1, keepdims=True)
    m2 = jnp.max(jnp.where(key == m1, -jnp.inf, key), axis=1, keepdims=True)
    g1 = jnp.max(m1, axis=0, keepdims=True)
    g2 = jnp.max(jnp.where(m1 == g1, m2, m1), axis=0, keepdims=True)

    def decode(g):
        code = lax.bitcast_convert_type(g, jnp.int32) & (S - 1)
        return jnp.clip(S - 1 - code[0, 0], 0, S - 1)

    i1 = decode(g1)
    i2 = decode(g2)

    c1 = i1 // B
    c2 = i2 // B
    c2 = jnp.where(c1 == c2, (c1 + 1) % NB, c2)
    lo = jnp.minimum(c1, c2)
    hi = jnp.maximum(c1, c2)

    def cp_out(blk, s):
        r = pl.ds(pl.multiple_of(blk * B, B), B)
        return pltpu.make_async_copy(o_buf.at[r], out_hbm.at[r], sem_o.at[0])

    def early_blk(s):
        o = s + (s >= lo).astype(jnp.int32)
        return o + (o >= hi).astype(jnp.int32)

    with _Scope('wwait'):
        for ci in range(len(F_CHUNKS)):
            for t in range(3):
                if (ci, t) != (len(F_CHUNKS) - 1, 2):
                    cp_w(ci, t).wait()
    for s in range(NB - 2):
        cp_out(early_blk(s), s).start()

    row16 = lax.broadcasted_iota(jnp.int32, (16, 128), 0)

    def pick(ref_rows):
        return jnp.where(row16 == 0, ref_rows(i1), jnp.where(row16 == 1, ref_rows(i2), 0.0))

    xc = jnp.concatenate([pick(lambda i, t=t: xc2_s[t, pl.ds(i, 1), :]) for t in range(NT)], axis=1)
    rs = pick(lambda i: st4[pl.ds(i, 1), :])[:, 0:1]
    mu = pick(lambda i: st1[pl.ds(i, 1), :] + st3[pl.ds(i, 1), :])[:, 0:1]
    h2 = xc * rs * par[6, 0:1] + par[7, 0:1]
    gate = jax.nn.sigmoid(jnp.sum(h2 * par[5, 0:1], axis=1, keepdims=True))
    h2b = h2.astype(bf16)

    acc = jnp.zeros((16, D), f32)
    with _Scope('mlp'):
        for ci, (f0, fn) in enumerate(F_CHUNKS):
            if ci == len(F_CHUNKS) - 1:
                cp_w(ci, 2).wait()
            gg = lax.dot_general(h2b, wg_buf[f0:f0 + fn, :], nt_dims, preferred_element_type=f32)
            uu = lax.dot_general(h2b, wu_buf[f0:f0 + fn, :], nt_dims, preferred_element_type=f32)
            act = (gg * jax.nn.sigmoid(gg) * uu).astype(bf16)
            acc = acc + jnp.dot(act, wd_buf[f0:f0 + fn, :], preferred_element_type=f32)
    o_sel = xc + mu + par[8, 0:1] * (h2 + acc * gate)

    row16d = lax.broadcasted_iota(jnp.int32, (16, D), 0)
    for t, idx in enumerate((i1, i2)):
        base = pl.multiple_of((idx // 16) * 16, 16)
        tile = o_buf[pl.ds(base, 16), :].astype(f32)
        tile = jnp.where(row16d == idx - base, o_sel[t:t + 1], tile)
        o_buf[pl.ds(base, 16), :] = tile.astype(bf16)
    cp_out(lo, NB - 2).start()
    cp_out(hi, NB - 1).start()


N_IN_SEM = 5 + NT + 2 * NKV + 1 + NQ + 3 * len(F_CHUNKS)


def _kernel(*refs):
    pl.run_scoped(lambda sem: _body(*refs, sem), pltpu.SemaphoreType.DMA((N_IN_SEM,)))
    out_hbm, o_buf, sem_o = refs[13], refs[-5], refs[-1]
    pltpu.make_async_copy(o_buf, out_hbm, sem_o.at[0]).wait()


@jax.jit
def pallas_adaLN_cond__ssm_conv_h3__moe_arch_mod__prompt_kernel(
    A_q, A_k, A_v, A_shift_k, A_ssm_k, A_ssm_D, B_x, B_w_r, B_w_gate, B_w_up, B_w_down, c, w_mod,
):
    del B_x
    args = (
        A_q.reshape(S, D), A_k.reshape(S, D), A_v.reshape(S, D), A_shift_k.T, A_ssm_k,
        A_ssm_D.reshape(NT, 128), B_w_r.reshape(NT, 128), B_w_gate.T, B_w_up.T, B_w_down,
        c, w_mod, jnp.asarray(_dft_consts(), bf16),
    )
    vm = pltpu.VMEM
    in_bufs = [vm(a.shape, a.dtype) for a in args]
    in_bufs[4] = vm((NT, NB, 128, B), bf16)
    scratch = in_bufs + [
        vm((NT, S + 8, 128), f32),
        vm((NT, NG, 2, 8, 128), f32),
        vm((NT, NB, 3, NG, 8, 128), f32),
        vm((NB, NG, 2, 8, 128), f32),
        vm((NB, NG, 2, 8, 128), f32),
        vm((NB, 2 * B, 128), bf16),
        vm((NB, 2 * B, 128), bf16),
        vm((NT, S, 128), f32),
        vm((NT, S, 128), f32),
        vm((NT, S, 128), f32),
        vm((NT, S, 128), f32),
        vm((NT, S, 128), f32),
        vm((S, 128), f32),
        vm((S, 128), f32),
        vm((S, 128), f32),
        vm((S, 128), f32),
        vm((S, 128), f32),
        vm((S, D), bf16),
        vm((9, 8, D), f32),
        vm((2, 8, 128), f32),
        pltpu.SMEM((4,), jnp.int32),
        pltpu.SemaphoreType.DMA((1,)),
    ]
    out = pl.pallas_call(
        _kernel,
        out_shape=jax.ShapeDtypeStruct((S, D), bf16),
        in_specs=[pl.BlockSpec(memory_space=pl.ANY)] * len(args),
        out_specs=pl.BlockSpec(memory_space=pl.ANY),
        scratch_shapes=scratch,
        compiler_params=pltpu.CompilerParams(vmem_limit_bytes=120 * 1024 * 1024),
        name="adaln_h3_mod",
    )(*args)
    return out.reshape(1, S, D)
```

```python
import math

import numpy as np
import jax
import jax.numpy as jnp
from jax import lax
import jax.experimental.pallas as pl
import jax.experimental.pallas.tpu as pltpu

S = 2048
D = 640
B = 128
NB = S // B
NT = D // 128
NG = B // 8
EPS = 1e-5
KV_CH = 256
NKV = S // KV_CH
HALO = 16
GPI = 4
F_CHUNKS = ((0, 512), (512, 512), (1024, 512), (1536, 192))
N_IN_SEM = 5 + NT + 2 * NKV + 2 + 3 * len(F_CHUNKS)

f32 = jnp.float32
bf16 = jnp.bfloat16
u32 = jnp.uint32


def _dft_consts():
    k = np.concatenate([np.arange(0, B, 2), np.arange(1, B, 2)]).astype(np.float64)
    n = np.arange(B, dtype=np.float64)
    th = 2.0 * np.pi * (k[:, None] + 0.5) * n[None, :] / (2 * B)
    fwd = np.stack([np.cos(th).reshape(NG, 8, B), -np.sin(th).reshape(NG, 8, B)], axis=1).reshape(2 * B, B)
    n2 = np.arange(B, 2 * B, dtype=np.float64)
    th2 = 2.0 * np.pi * (k[None, :] + 0.5) * n2[:, None] / (2 * B)
    inv = np.stack([np.cos(th2).reshape(B, NG, 8), -np.sin(th2).reshape(B, NG, 8)], axis=2).reshape(B, 2 * B) / B
    inv = np.concatenate([inv[:, :B], inv[:, B:]], axis=0)
    mat = np.concatenate([fwd, inv], axis=0).astype(np.float32).astype(bf16)
    half = mat.view(np.uint16).astype(np.uint32)
    return half[0::2] | (half[1::2] << 16)


def _rs(ssq):
    return jnp.exp2(jnp.log(ssq + D * EPS) * (-0.5 / math.log(2.0)))


def _body(q_hbm, k_hbm, v_hbm, sk_hbm, h_hbm, dd_hbm, wr_hbm, wg_hbm, wu_hbm, wd_hbm,
          c_hbm, wm_hbm, fc_hbm,
          out_hbm,
          q_buf, k_buf, v_buf, sk_buf, h_buf, dd_buf, wr_buf, wg_buf, wu_buf, wd_buf,
          c_buf, wm_buf, fc_buf,
          prev, u_s, hp, g_a, g_b, y_a, y_b, y_lo, y_hi, xc_s, x2_s, xc2_s,
          st1, st2, st3, st4, st5, o_buf, par, r_s, zs,
          sem_o, sem):
    o_small, o_h, o_k, o_v, o_wm, o_q, o_w = [int(o) for o in np.cumsum([0, 5, NT, NKV, NKV, 1, 1])]
    small = [(fc_hbm, fc_buf), (sk_hbm, sk_buf), (dd_hbm, dd_buf), (c_hbm, c_buf), (wr_hbm, wr_buf)]
    cp_small = [pltpu.make_async_copy(s, d, sem.at[o_small + i]) for i, (s, d) in enumerate(small)]

    def cp_rows(src, dst, off, i, rows):
        return pltpu.make_async_copy(src.at[pl.ds(i * rows, rows)], dst.at[pl.ds(i * rows, rows)], sem.at[off + i])

    def cp_k(i):
        return pltpu.make_async_copy(k_hbm.at[pl.ds(i * KV_CH, KV_CH)],
                                     k_buf.at[pl.ds(HALO + i * KV_CH, KV_CH)], sem.at[o_k + i])

    def cp_h(j):
        return cp_rows(h_hbm, h_buf, o_h, j, 128)

    cp_wm = pltpu.make_async_copy(wm_hbm, wm_buf, sem.at[o_wm])
    cp_q = pltpu.make_async_copy(q_hbm, q_buf, sem.at[o_q])

    def cp_w(ci, t):
        f0, fn = F_CHUNKS[ci]
        src, dst = ((wg_hbm, wg_buf), (wu_hbm, wu_buf), (wd_hbm, wd_buf))[t]
        return pltpu.make_async_copy(src.at[pl.ds(f0, fn)], dst.at[pl.ds(f0, fn)], sem.at[o_w + ci * 3 + t])

    cp_small[0].start()
    cp_h(0).start()
    for c in cp_small[1:]:
        c.start()
    for i in range(NKV):
        cp_k(i).start()
        cp_rows(v_hbm, v_buf, o_v, i, KV_CH).start()
    for j in range(1, NT):
        cp_h(j).start()
    cp_wm.start()
    cp_q.start()
    for ci in range(len(F_CHUNKS)):
        for t in range(3):
            cp_w(ci, t).start()

    for t in range(4):
        zs[t] = 0
    for j in range(NT):
        prev[j] = jnp.zeros((NG, 2, 8, 128), f32)
    r_s[...] = jnp.zeros((2, 8, 128), f32)
    k_buf[0:HALO, :] = jnp.zeros((HALO, D), bf16)

    nt_dims = (((1,), (1,)), ((), ()))
    inv_d = 1.0 / D

    def as_bf16(w):
        return pltpu.bitcast(w, bf16)

    def f_fwd():
        return as_bf16(fc_buf[0:B, :])

    def h_tile(j, m):
        return h_buf[pl.ds(j * 128, 128), pl.ds(pl.multiple_of(m * B, B), B)]

    def stage_r(j, m):
        hp[m] = pltpu.bitcast(h_tile(j, m), u32)

    def stage_h(tile, m, g_dst):
        hh = lax.dot_general(f_fwd(), tile, nt_dims, preferred_element_type=f32)
        g_dst[m] = hh.reshape(NG, 2, 8, 128)

    def fix_d(j, g_dst):
        dj = dd_buf[j:j + 1, :].astype(f32)[None]
        g_dst[0, :, 0] = g_dst[0, :, 0] + dj

    def stage_i(j, a, y_src):
        rows = pl.ds(pl.multiple_of(a * B, B), B)
        hb = B // 2
        y_lo[j, rows, :] = jnp.dot(as_bf16(fc_buf[B:B + hb, :]), as_bf16(y_src[a, 0:hb]),
                                   preferred_element_type=f32)
        y_hi[j, rows, :] = jnp.dot(as_bf16(fc_buf[B + hb:, :]), as_bf16(y_src[a, hb:]),
                                   preferred_element_type=f32)

    def stage_c(j, g, g_src, y_dst):
        for half in range(2):
            gg = jnp.clip(g + zs[half], 0, NG - 1)
            g2 = jnp.clip(g + zs[2 + half], 0, NG - 1)
            lo = half * 8
            n_in = lo + 8
            res = []
            for comp in range(3):
                acc = [None] * 8 if comp == 0 else list(res[0])
                v = {}
                for jj in range(n_in):
                    u = u_s[j, jj, comp, gg]
                    for o in range(8):
                        m = lo + o - jj
                        if m < 0:
                            continue
                        if m not in v:
                            if comp == 0:
                                v[m] = g_src[m, g2, 0] + g_src[m, g2, 1]
                            else:
                                v[m] = g_src[m, gg, comp - 1]
                        p = u * v[m]
                        if acc[o] is None:
                            acc[o] = p
                        elif comp == 2:
                            acc[o] = acc[o] - p
                        else:
                            acc[o] = acc[o] + p
                res.append(acc)
            for o in range(8):
                packed = jnp.concatenate([res[2][o], res[1][o]], axis=0).astype(bf16)
                y_dst[lo + o, pl.ds(pl.multiple_of(g * 8, 8), 8), :] = pltpu.bitcast(packed, u32)

    def lanes(t):
        return slice(t * 128, (t + 1) * 128)

    def rsum(xs):
        s = xs[0]
        for x in xs[1:]:
            s = s + x
        return jnp.broadcast_to(jnp.sum(s, axis=1, keepdims=True), (8, 128))

    def grp(r0, gi):
        return pl.ds(pl.multiple_of(r0 + gi * 8, 8), 8)

    def stage_a(r0, nrows):
        for gi in range(nrows // 8):
            rows = grp(r0, gi)
            st1[rows, :] = rsum([q_buf[rows, lanes(t)].astype(f32) for t in range(NT)]) * inv_d

    def stage_b(r0, nrows):
        for gi in range(nrows // 8):
            rows = grp(r0, gi)
            mu = st1[rows, :]
            sq = []
            for t in range(NT):
                xc = q_buf[rows, lanes(t)].astype(f32) - mu
                xc_s[t, rows, :] = xc
                sq.append(xc * xc)
            st2[rows, :] = _rs(rsum(sq))

    def stage_x(r0):
        for gi in range(NG):
            rows = grp(r0, gi)
            rs = st2[rows, :]
            xs = []
            for t in range(NT):
                xc = xc_s[t, rows, :]
                y = y_lo[t, rows, :] + y_hi[t, rows, :]
                x2 = ((xc * rs) * par[0, :, lanes(t)] + par[1, :, lanes(t)]) * y + xc
                x2_s[t, rows, :] = x2
                xs.append(x2)
            st3[rows, :] = rsum(xs) * inv_d

    def stage_d(r0):
        for gi in range(NG):
            rows = grp(r0, gi)
            mu = st3[rows, :]
            sq, rd = [], []
            for t in range(NT):
                xc = x2_s[t, rows, :] - mu
                xc2_s[t, rows, :] = xc
                sq.append(xc * xc)
                rd.append(xc * par[4, :, lanes(t)])
            rs = _rs(rsum(sq))
            st4[rows, :] = rs
            st5[rows, :] = rsum(rd) * rs

    lane = lax.broadcasted_iota(jnp.int32, (8, 128), 1)

    def stage_e(a, r0):
        rblk = r_s[a // 8]
        lane_rel = lane - (a % 8) * NG
        for gi in range(NG):
            rows = grp(r0, gi)
            rs = st4[rows, :]
            mu = st1[rows, :] + st3[rows, :]
            rblk = jnp.where(lane_rel == gi, st5[rows, :], rblk)
            for t in range(NT):
                xc = xc2_s[t, rows, :]
                out = (xc * rs) * par[2, :, lanes(t)] + xc + (par[3, :, lanes(t)] + mu)
                o_buf[rows, lanes(t)] = out.astype(bf16)
        r_s[a // 8] = rblk

    def build_par():
        cf = c_buf[...].astype(f32)
        cs = (cf * jax.nn.sigmoid(cf)).astype(bf16)
        mod = jnp.dot(jnp.broadcast_to(cs, (16, D)), wm_buf[...], preferred_element_type=f32)[0:8]
        sa, ca, ga, sb, cb, gb = [mod[:, i * D:(i + 1) * D] for i in range(6)]
        wr = jnp.concatenate([jnp.broadcast_to(wr_buf[t:t + 1, :].astype(f32), (8, 128))
                              for t in range(NT)], axis=1)
        sqd = math.sqrt(D)
        par[0] = ga * (1.0 + ca) * sqd
        par[1] = ga * sa
        par[2] = gb * (1.0 + cb) * sqd
        par[3] = gb * sb
        par[4] = (1.0 + cb) * wr
        par[5] = wr
        par[6] = (1.0 + cb) * sqd
        par[7] = sb
        par[8] = gb

    cp_small[0].wait()
    cp_h(0).wait()

    def h0_body(i, c):
        for t in range(4):
            stage_h(h_tile(0, i * 4 + t), i * 4 + t, g_a)
        return c
    lax.fori_loop(0, NB // 4, h0_body, 0)
    for c in cp_small[1:]:
        c.wait()
    fix_d(0, g_a)

    def p_body(i, c):
        cp_k(i).wait()
        cp_rows(v_hbm, v_buf, o_v, i, KV_CH).wait()
        sk = sk_buf[...].astype(f32)
        nblk = KV_CH // B
        for j in range(NT):
            ls = lanes(j)
            for t in range(nblk):
                a = i * nblk + t
                r0 = pl.multiple_of(a * B, B)
                kw = k_buf[pl.ds(r0 + HALO - 8, B + 8), ls].astype(f32)
                ks = kw[8:] * sk[0:1, ls]
                for t2 in range(1, 4):
                    ks = ks + kw[8 - t2:B + 8 - t2] * sk[t2:t2 + 1, ls]
                kv = (ks * v_buf[pl.ds(r0, B), ls].astype(f32)).astype(bf16)
                x = jnp.dot(f_fwd(), kv, preferred_element_type=f32).reshape(NG, 2, 8, 128)
                p = prev[j] if t == 0 else xprev
                xprev = x
                if t == nblk - 1:
                    prev[j] = x
                hb = NG // 2
                wr_ = jnp.concatenate([p[:hb, 0] + x[:hb, 1], p[hb:, 0] - x[hb:, 1]], axis=0)
                wi_ = jnp.concatenate([p[:hb, 1] - x[:hb, 0], p[hb:, 1] + x[hb:, 0]], axis=0)
                u_s[j, a, 0] = wr_
                u_s[j, a, 1] = wi_ - wr_
                u_s[j, a, 2] = wr_ + wi_
        return c
    lax.fori_loop(0, NKV, p_body, 0)

    gs = (g_a, g_b)
    ys = (y_a, y_b)
    n_it = NG // GPI
    for j in range(NT):
        if j + 1 < NT:
            cp_h(j + 1).wait()
            for m in range(NB):
                stage_r(j + 1, m)

        def c_body(i, c, j=j):
            for t in range(GPI):
                g = i * GPI + t
                if j + 1 < NT:
                    stage_h(as_bf16(hp[g]), g, gs[(j + 1) % 2])
                if j > 0:
                    stage_i(j - 1, g, ys[(j - 1) % 2])
                stage_c(j, g, gs[j % 2], ys[j % 2])
            return c
        lax.fori_loop(0, n_it, c_body, 0)
        if j + 1 < NT:
            fix_d(j + 1, gs[(j + 1) % 2])

    y_last = ys[(NT - 1) % 2]
    cp_wm.wait()
    cp_q.wait()
    build_par()
    for a in range(3):
        stage_i(NT - 1, a, y_last)
    stage_a(0, S)
    stage_b(0, S)
    stage_x(0)
    stage_x(B)
    stage_d(0)

    def e_body(a, c):
        stage_i(NT - 1, a + 3, y_last)
        stage_x((a + 2) * B)
        stage_d((a + 1) * B)
        stage_e(a, a * B)
        return c
    lax.fori_loop(0, NB - 3, e_body, 0)
    stage_x((NB - 1) * B)
    stage_d((NB - 2) * B)
    stage_e(NB - 3, (NB - 3) * B)
    stage_d((NB - 1) * B)
    stage_e(NB - 2, (NB - 2) * B)
    stage_e(NB - 1, (NB - 1) * B)

    rall = r_s[...].reshape(16, 128)
    sub = lax.broadcasted_iota(jnp.int32, (16, 128), 0)
    ln = lax.broadcasted_iota(jnp.int32, (16, 128), 1)
    ridx = (sub // 8) * (S // 2) + ln * 8 + (sub % 8)
    bits = lax.bitcast_convert_type(rall, jnp.int32)
    bits = jnp.where((bits & jnp.int32(0x7F800000)) == 0, jnp.int32(0x00800000), bits)
    code = jnp.where(bits < 0, ridx, S - 1 - ridx)
    key = lax.bitcast_convert_type((bits & jnp.int32(-S)) | code, f32)
    m1 = jnp.max(key, axis=1, keepdims=True)
    m2 = jnp.max(jnp.where(key == m1, -jnp.inf, key), axis=1, keepdims=True)
    g1 = jnp.max(m1, axis=0, keepdims=True)
    g2 = jnp.max(jnp.where(m1 == g1, m2, m1), axis=0, keepdims=True)

    def decode(g):
        gb = lax.bitcast_convert_type(g, jnp.int32)
        c = gb & (S - 1)
        return jnp.clip(jnp.where(gb < 0, c, S - 1 - c)[0, 0], 0, S - 1)

    i1 = decode(g1)
    i2 = decode(g2)

    c1 = i1 // B
    c2 = i2 // B
    c2 = jnp.where(c1 == c2, (c1 + 1) % NB, c2)
    lo = jnp.minimum(c1, c2)
    hi = jnp.maximum(c1, c2)

    def cp_out(blk):
        r = pl.ds(pl.multiple_of(blk * B, B), B)
        return pltpu.make_async_copy(o_buf.at[r], out_hbm.at[r], sem_o.at[0])

    def early_blk(s):
        o = s + (s >= lo).astype(jnp.int32)
        return o + (o >= hi).astype(jnp.int32)

    for ci in range(len(F_CHUNKS)):
        for t in range(3):
            if (ci, t) != (len(F_CHUNKS) - 1, 2):
                cp_w(ci, t).wait()
    for s in range(NB - 2):
        cp_out(early_blk(s)).start()

    row16 = lax.broadcasted_iota(jnp.int32, (16, 128), 0)

    def pick(ref_rows):
        return jnp.where(row16 == 0, ref_rows(i1), jnp.where(row16 == 1, ref_rows(i2), 0.0))

    xc = jnp.concatenate([pick(lambda i, t=t: xc2_s[t, pl.ds(i, 1), :]) for t in range(NT)], axis=1)
    rs = pick(lambda i: st4[pl.ds(i, 1), :])[:, 0:1]
    mu = pick(lambda i: st1[pl.ds(i, 1), :] + st3[pl.ds(i, 1), :])[:, 0:1]
    h2 = xc * rs * par[6, 0:1] + par[7, 0:1]
    gate = jax.nn.sigmoid(jnp.sum(h2 * par[5, 0:1], axis=1, keepdims=True))
    h2b = h2.astype(bf16)

    acc = jnp.zeros((16, D), f32)
    for ci, (f0, fn) in enumerate(F_CHUNKS):
        if ci == len(F_CHUNKS) - 1:
            cp_w(ci, 2).wait()
        gg = lax.dot_general(h2b, wg_buf[f0:f0 + fn, :], nt_dims, preferred_element_type=f32)
        uu = lax.dot_general(h2b, wu_buf[f0:f0 + fn, :], nt_dims, preferred_element_type=f32)
        act = (gg * jax.nn.sigmoid(gg) * uu).astype(bf16)
        acc = acc + jnp.dot(act, wd_buf[f0:f0 + fn, :], preferred_element_type=f32)
    o_sel = xc + mu + par[8, 0:1] * (h2 + acc * gate)

    row16d = lax.broadcasted_iota(jnp.int32, (16, D), 0)
    for t, idx in enumerate((i1, i2)):
        base = pl.multiple_of((idx // 16) * 16, 16)
        tile = o_buf[pl.ds(base, 16), :].astype(f32)
        tile = jnp.where(row16d == idx - base, o_sel[t:t + 1], tile)
        o_buf[pl.ds(base, 16), :] = tile.astype(bf16)
    cp_out(lo).start()
    cp_out(hi).start()


def _kernel(*refs):
    pl.run_scoped(lambda sem: _body(*refs, sem), pltpu.SemaphoreType.DMA((N_IN_SEM,)))
    out_hbm, o_buf, sem_o = refs[13], refs[-5], refs[-1]
    pltpu.make_async_copy(o_buf, out_hbm, sem_o.at[0]).wait()


@jax.jit
def pallas_adaLN_cond__ssm_conv_h3__moe_arch_mod__prompt_kernel(
    A_q, A_k, A_v, A_shift_k, A_ssm_k, A_ssm_D, B_x, B_w_r, B_w_gate, B_w_up, B_w_down, c, w_mod,
):
    del B_x
    args = (
        A_q.reshape(S, D), A_k.reshape(S, D), A_v.reshape(S, D), A_shift_k.T, A_ssm_k,
        A_ssm_D.reshape(NT, 128), B_w_r.reshape(NT, 128), B_w_gate.T, B_w_up.T, B_w_down,
        c, w_mod, jnp.asarray(_dft_consts()),
    )
    vm = pltpu.VMEM
    in_bufs = [vm(a.shape, a.dtype) for a in args]
    in_bufs[1] = vm((HALO + S, D), bf16)
    scratch = in_bufs + [
        vm((NT, NG, 2, 8, 128), f32),
        vm((NT, NB, 3, NG, 8, 128), f32),
        vm((NB, 64, 128), u32),
        vm((NB, NG, 2, 8, 128), f32),
        vm((NB, NG, 2, 8, 128), f32),
        vm((NB, B, 128), u32),
        vm((NB, B, 128), u32),
        vm((NT, S, 128), f32),
        vm((NT, S, 128), f32),
        vm((NT, S, 128), f32),
        vm((NT, S, 128), f32),
        vm((NT, S, 128), f32),
        vm((S, 128), f32),
        vm((S, 128), f32),
        vm((S, 128), f32),
        vm((S, 128), f32),
        vm((S, 128), f32),
        vm((S, D), bf16),
        vm((9, 8, D), f32),
        vm((2, 8, 128), f32),
        pltpu.SMEM((4,), jnp.int32),
        pltpu.SemaphoreType.DMA((1,)),
    ]
    out = pl.pallas_call(
        _kernel,
        out_shape=jax.ShapeDtypeStruct((S, D), bf16),
        in_specs=[pl.BlockSpec(memory_space=pl.ANY)] * len(args),
        out_specs=pl.BlockSpec(memory_space=pl.ANY),
        scratch_shapes=scratch,
        compiler_params=pltpu.CompilerParams(vmem_limit_bytes=120 * 1024 * 1024),
        name="adaln_h3_mod",
    )(*args)
    return out.reshape(1, S, D)
```

```python
import math

import numpy as np
import jax
import jax.numpy as jnp
from jax import lax
import jax.experimental.pallas as pl
import jax.experimental.pallas.tpu as pltpu

S = 2048
D = 640
B = 128
NB = S // B
NT = D // 128
NG = B // 8
EPS = 1e-5
KV_CH = 256
NKV = S // KV_CH
HALO = 16
NREG = 4
OROWS = S // (NREG * NB)
GPI = 4
F_CHUNKS = ((0, 512), (512, 512), (1024, 384), (1408, 320))
N_IN_SEM = 5 + NT + 2 * NKV + 2 + 3 * len(F_CHUNKS)

f32 = jnp.float32
bf16 = jnp.bfloat16
u32 = jnp.uint32


def _dft_consts():
    k = np.concatenate([np.arange(0, B, 2), np.arange(1, B, 2)]).astype(np.float64)
    n = np.arange(B, dtype=np.float64)
    th = 2.0 * np.pi * (k[:, None] + 0.5) * n[None, :] / (2 * B)
    fwd = np.stack([np.cos(th).reshape(NG, 8, B), -np.sin(th).reshape(NG, 8, B)], axis=1).reshape(2 * B, B)
    n2 = np.arange(B, 2 * B, dtype=np.float64)
    th2 = 2.0 * np.pi * (k[None, :] + 0.5) * n2[:, None] / (2 * B)
    inv = np.stack([np.cos(th2).reshape(B, NG, 8), -np.sin(th2).reshape(B, NG, 8)], axis=2).reshape(B, 2 * B) / B
    inv = np.concatenate([inv[:, :B], inv[:, B:]], axis=0)
    mat = np.concatenate([fwd, inv], axis=0).astype(np.float32).astype(bf16)
    half = mat.view(np.uint16).astype(np.uint32)
    return half[0::2] | (half[1::2] << 16)


def _rs(ssq):
    return jnp.exp2(jnp.log(ssq + D * EPS) * (-0.5 / math.log(2.0)))


def _body(q_hbm, k_hbm, v_hbm, sk_hbm, h_hbm, dd_hbm, wr_hbm, wg_hbm, wu_hbm, wd_hbm,
          c_hbm, wm_hbm, fc_hbm,
          out_hbm,
          q_buf, k_buf, v_buf, sk_buf, h_buf, dd_buf, wr_buf, wg_buf, wu_buf, wd_buf,
          c_buf, wm_buf, fc_buf,
          prev, u_s, hp, g_a, g_b, y_a, y_b, y_lo, y_hi, xc_s, x2_s, xc2_s,
          st1, st2, st3, st4, st5, o_buf, par, r_s, zs,
          sem_o, sem):
    o_small, o_h, o_k, o_v, o_wm, o_q, o_w = [int(o) for o in np.cumsum([0, 5, NT, NKV, NKV, 1, 1])]
    small = [(fc_hbm, fc_buf), (sk_hbm, sk_buf), (dd_hbm, dd_buf), (c_hbm, c_buf), (wr_hbm, wr_buf)]
    cp_small = [pltpu.make_async_copy(s, d, sem.at[o_small + i]) for i, (s, d) in enumerate(small)]

    def cp_rows(src, dst, off, i, rows):
        return pltpu.make_async_copy(src.at[pl.ds(i * rows, rows)], dst.at[pl.ds(i * rows, rows)], sem.at[off + i])

    def cp_k(i):
        return pltpu.make_async_copy(k_hbm.at[pl.ds(i * KV_CH, KV_CH)],
                                     k_buf.at[pl.ds(HALO + i * KV_CH, KV_CH)], sem.at[o_k + i])

    def cp_h(j):
        return cp_rows(h_hbm, h_buf, o_h, j, 128)

    cp_wm = pltpu.make_async_copy(wm_hbm, wm_buf, sem.at[o_wm])
    cp_q = pltpu.make_async_copy(q_hbm, q_buf, sem.at[o_q])

    def cp_w(ci, t):
        f0, fn = F_CHUNKS[ci]
        src, dst = ((wg_hbm, wg_buf), (wu_hbm, wu_buf), (wd_hbm, wd_buf))[t]
        return pltpu.make_async_copy(src.at[pl.ds(f0, fn)], dst.at[pl.ds(f0, fn)], sem.at[o_w + ci * 3 + t])

    cp_small[0].start()
    cp_h(0).start()
    for c in cp_small[1:]:
        c.start()
    for i in range(NKV):
        cp_k(i).start()
        cp_rows(v_hbm, v_buf, o_v, i, KV_CH).start()
    for j in range(1, NT):
        cp_h(j).start()
    cp_wm.start()
    cp_q.start()
    for ci in range(len(F_CHUNKS)):
        for t in range(3):
            cp_w(ci, t).start()

    for t in range(4):
        zs[t] = 0
    for j in range(NT):
        prev[j] = jnp.zeros((NG, 2, 8, 128), f32)
    r_s[...] = jnp.zeros((2, 8, 128), f32)
    k_buf[0:HALO, :] = jnp.zeros((HALO, D), bf16)

    nt_dims = (((1,), (1,)), ((), ()))
    inv_d = 1.0 / D

    def as_bf16(w):
        return pltpu.bitcast(w, bf16)

    def f_fwd():
        return as_bf16(fc_buf[0:B, :])

    def h_tile(j, m):
        return h_buf[pl.ds(j * 128, 128), pl.ds(pl.multiple_of(m * B, B), B)]

    def stage_r(j, m):
        hp[m] = pltpu.bitcast(h_tile(j, m), u32)

    def stage_h(tile, m, g_dst):
        hh = lax.dot_general(f_fwd(), tile, nt_dims, preferred_element_type=f32)
        g_dst[m] = hh.reshape(NG, 2, 8, 128)

    def fix_d(j, g_dst):
        dj = dd_buf[j:j + 1, :].astype(f32)[None]
        g_dst[0, :, 0] = g_dst[0, :, 0] + dj

    def stage_i(j, a, y_src):
        rows = pl.ds(pl.multiple_of(a * B, B), B)
        hb = B // 2
        y_lo[j, rows, :] = jnp.dot(as_bf16(fc_buf[B:B + hb, :]), as_bf16(y_src[a, 0:hb]),
                                   preferred_element_type=f32)
        y_hi[j, rows, :] = jnp.dot(as_bf16(fc_buf[B + hb:, :]), as_bf16(y_src[a, hb:]),
                                   preferred_element_type=f32)

    def stage_c(j, g, g_src, y_dst):
        for half in range(2):
            gg = jnp.clip(g + zs[half], 0, NG - 1)
            g2 = jnp.clip(g + zs[2 + half], 0, NG - 1)
            lo = half * 8
            n_in = lo + 8
            res = []
            for comp in range(3):
                acc = [None] * 8 if comp == 0 else list(res[0])
                v = {}
                for jj in range(n_in):
                    u = u_s[j, jj, comp, gg]
                    for o in range(8):
                        m = lo + o - jj
                        if m < 0:
                            continue
                        if m not in v:
                            if comp == 0:
                                v[m] = g_src[m, g2, 0] + g_src[m, g2, 1]
                            else:
                                v[m] = g_src[m, gg, comp - 1]
                        p = u * v[m]
                        if acc[o] is None:
                            acc[o] = p
                        elif comp == 2:
                            acc[o] = acc[o] - p
                        else:
                            acc[o] = acc[o] + p
                res.append(acc)
                if comp > 0:
                    r4 = pl.ds(pl.multiple_of(g * 8 + 4 * (2 - comp), 4), 4)
                    for o in range(8):
                        y_dst[lo + o, r4, :] = pltpu.bitcast(acc[o].astype(bf16), u32)

    def lanes(t):
        return slice(t * 128, (t + 1) * 128)

    def rsum(xs):
        s = xs[0]
        for x in xs[1:]:
            s = s + x
        return jnp.broadcast_to(jnp.sum(s, axis=1, keepdims=True), (8, 128))

    def grp(r0, gi):
        return pl.ds(pl.multiple_of(r0 + gi * 8, 8), 8)

    def stage_a(r0, nrows):
        for gi in range(nrows // 8):
            rows = grp(r0, gi)
            st1[rows, :] = rsum([q_buf[rows, lanes(t)].astype(f32) for t in range(NT)]) * inv_d

    def stage_b(r0, nrows):
        for gi in range(nrows // 8):
            rows = grp(r0, gi)
            mu = st1[rows, :]
            sq = []
            for t in range(NT):
                xc = q_buf[rows, lanes(t)].astype(f32) - mu
                xc_s[t, rows, :] = xc
                sq.append(xc * xc)
            st2[rows, :] = _rs(rsum(sq))

    def stage_x(r0):
        for gi in range(NG):
            rows = grp(r0, gi)
            rs = st2[rows, :]
            xs = []
            for t in range(NT):
                xc = xc_s[t, rows, :]
                y = y_lo[t, rows, :] + y_hi[t, rows, :]
                x2 = ((xc * rs) * par[0, :, lanes(t)] + par[1, :, lanes(t)]) * y + xc
                x2_s[t, rows, :] = x2
                xs.append(x2)
            st3[rows, :] = rsum(xs) * inv_d

    def stage_d(r0):
        for gi in range(NG):
            rows = grp(r0, gi)
            mu = st3[rows, :]
            sq, rd = [], []
            for t in range(NT):
                xc = x2_s[t, rows, :] - mu
                xc2_s[t, rows, :] = xc
                sq.append(xc * xc)
                rd.append(xc * par[4, :, lanes(t)])
            rs = _rs(rsum(sq))
            st4[rows, :] = rs
            st5[rows, :] = rsum(rd) * rs

    lane = lax.broadcasted_iota(jnp.int32, (8, 128), 1)

    def stage_e(a, r0):
        rblk = r_s[a // 8]
        lane_rel = lane - (a % 8) * NG
        for gi in range(NG):
            rows = grp(r0, gi)
            rs = st4[rows, :]
            mu = st1[rows, :] + st3[rows, :]
            rblk = jnp.where(lane_rel == gi, st5[rows, :], rblk)
            for t in range(NT):
                xc = xc2_s[t, rows, :]
                out = (xc * rs) * par[2, :, lanes(t)] + xc + (par[3, :, lanes(t)] + mu)
                o_buf[a // NREG, (a % NREG) * NREG + gi // 4, (gi % 4) * 8:(gi % 4) * 8 + 8, lanes(t)] = (
                    out.astype(bf16))
        r_s[a // 8] = rblk

    def build_par():
        cf = c_buf[...].astype(f32)
        cs = (cf * jax.nn.sigmoid(cf)).astype(bf16)
        mod = jnp.dot(jnp.broadcast_to(cs, (16, D)), wm_buf[...], preferred_element_type=f32)[0:8]
        sa, ca, ga, sb, cb, gb = [mod[:, i * D:(i + 1) * D] for i in range(6)]
        wr = jnp.concatenate([jnp.broadcast_to(wr_buf[t:t + 1, :].astype(f32), (8, 128))
                              for t in range(NT)], axis=1)
        sqd = math.sqrt(D)
        par[0] = ga * (1.0 + ca) * sqd
        par[1] = ga * sa
        par[2] = gb * (1.0 + cb) * sqd
        par[3] = gb * sb
        par[4] = (1.0 + cb) * wr
        par[5] = wr
        par[6] = (1.0 + cb) * sqd
        par[7] = sb
        par[8] = gb

    cp_small[0].wait()
    cp_h(0).wait()

    def h0_body(i, c):
        for t in range(4):
            stage_h(h_tile(0, i * 4 + t), i * 4 + t, g_a)
        return c
    lax.fori_loop(0, NB // 4, h0_body, 0)
    for c in cp_small[1:]:
        c.wait()
    fix_d(0, g_a)

    def p_body(i, c):
        cp_k(i).wait()
        cp_rows(v_hbm, v_buf, o_v, i, KV_CH).wait()
        sk = sk_buf[...].astype(f32)
        nblk = KV_CH // B
        for j in range(NT):
            ls = lanes(j)
            for t in range(nblk):
                a = i * nblk + t
                r0 = pl.multiple_of(a * B, B)
                kw = k_buf[pl.ds(r0 + HALO - 8, B + 8), ls].astype(f32)
                ks = kw[8:] * sk[0:1, ls]
                for t2 in range(1, 4):
                    ks = ks + kw[8 - t2:B + 8 - t2] * sk[t2:t2 + 1, ls]
                kv = (ks * v_buf[pl.ds(r0, B), ls].astype(f32)).astype(bf16)
                x = jnp.dot(f_fwd(), kv, preferred_element_type=f32).reshape(NG, 2, 8, 128)
                p = prev[j] if t == 0 else xprev
                xprev = x
                if t == nblk - 1:
                    prev[j] = x
                hb = NG // 2
                wr_ = jnp.concatenate([p[:hb, 0] + x[:hb, 1], p[hb:, 0] - x[hb:, 1]], axis=0)
                wi_ = jnp.concatenate([p[:hb, 1] - x[:hb, 0], p[hb:, 1] + x[hb:, 0]], axis=0)
                u_s[j, a, 0] = wr_
                u_s[j, a, 1] = wi_ - wr_
                u_s[j, a, 2] = wr_ + wi_
        return c
    lax.fori_loop(0, NKV, p_body, 0)

    gs = (g_a, g_b)
    ys = (y_a, y_b)
    n_it = NG // GPI
    for j in range(NT):
        if j + 1 < NT:
            cp_h(j + 1).wait()
            for m in range(NB):
                stage_r(j + 1, m)

        def c_body(i, c, j=j):
            for t in range(GPI):
                g = i * GPI + t
                if j + 1 < NT:
                    stage_h(as_bf16(hp[g]), g, gs[(j + 1) % 2])
                if j > 0:
                    stage_i(j - 1, g, ys[(j - 1) % 2])
                stage_c(j, g, gs[j % 2], ys[j % 2])
            return c
        lax.fori_loop(0, n_it, c_body, 0)
        if j + 1 < NT:
            fix_d(j + 1, gs[(j + 1) % 2])

    y_last = ys[(NT - 1) % 2]
    cp_wm.wait()
    cp_q.wait()
    build_par()
    for a in range(3):
        stage_i(NT - 1, a, y_last)
    stage_a(0, S)
    stage_b(0, S)
    stage_x(0)
    stage_x(B)
    stage_d(0)

    def e_body(a, c):
        stage_i(NT - 1, a + 3, y_last)
        stage_x((a + 2) * B)
        stage_d((a + 1) * B)
        stage_e(a, a * B)
        return c
    lax.fori_loop(0, NB - 3, e_body, 0)
    stage_x((NB - 1) * B)
    stage_d((NB - 2) * B)
    stage_e(NB - 3, (NB - 3) * B)
    stage_d((NB - 1) * B)
    stage_e(NB - 2, (NB - 2) * B)
    stage_e(NB - 1, (NB - 1) * B)

    rall = r_s[...].reshape(16, 128)
    sub = lax.broadcasted_iota(jnp.int32, (16, 128), 0)
    ln = lax.broadcasted_iota(jnp.int32, (16, 128), 1)
    ridx = (sub // 8) * (S // 2) + ln * 8 + (sub % 8)
    bits = lax.bitcast_convert_type(rall, jnp.int32)
    bits = jnp.where((bits & jnp.int32(0x7F800000)) == 0, jnp.int32(0x00800000), bits)
    code = jnp.where(bits < 0, ridx, S - 1 - ridx)
    key = lax.bitcast_convert_type((bits & jnp.int32(-S)) | code, f32)
    m1 = jnp.max(key, axis=1, keepdims=True)
    m2 = jnp.max(jnp.where(key == m1, -jnp.inf, key), axis=1, keepdims=True)
    g1 = jnp.max(m1, axis=0, keepdims=True)
    g2 = jnp.max(jnp.where(m1 == g1, m2, m1), axis=0, keepdims=True)

    def decode(g):
        gb = lax.bitcast_convert_type(g, jnp.int32)
        c = gb & (S - 1)
        return jnp.clip(jnp.where(gb < 0, c, S - 1 - c)[0, 0], 0, S - 1)

    i1 = decode(g1)
    i2 = decode(g2)

    c1 = (i1 % (S // NREG)) // OROWS
    c2 = (i2 % (S // NREG)) // OROWS
    c2 = jnp.where(c1 == c2, (c1 + 1) % NB, c2)
    lo = jnp.minimum(c1, c2)
    hi = jnp.maximum(c1, c2)

    def cp_out(blk):
        return pltpu.make_async_copy(o_buf.at[:, blk], out_hbm.at[:, blk], sem_o.at[0])

    def early_blk(s):
        o = s + (s >= lo).astype(jnp.int32)
        return o + (o >= hi).astype(jnp.int32)

    for ci in range(len(F_CHUNKS)):
        for t in range(3):
            if (ci, t) != (len(F_CHUNKS) - 1, 2):
                cp_w(ci, t).wait()
    for s in range(NB - 2):
        cp_out(early_blk(s)).start()

    row16 = lax.broadcasted_iota(jnp.int32, (16, 128), 0)

    def pick(ref_rows):
        return jnp.where(row16 == 0, ref_rows(i1), jnp.where(row16 == 1, ref_rows(i2), 0.0))

    xc = jnp.concatenate([pick(lambda i, t=t: xc2_s[t, pl.ds(i, 1), :]) for t in range(NT)], axis=1)
    rs = pick(lambda i: st4[pl.ds(i, 1), :])[:, 0:1]
    mu = pick(lambda i: st1[pl.ds(i, 1), :] + st3[pl.ds(i, 1), :])[:, 0:1]
    h2 = xc * rs * par[6, 0:1] + par[7, 0:1]
    gate = jax.nn.sigmoid(jnp.sum(h2 * par[5, 0:1], axis=1, keepdims=True))
    h2b = h2.astype(bf16)

    acc = jnp.zeros((16, D), f32)
    for ci, (f0, fn) in enumerate(F_CHUNKS):
        if ci == len(F_CHUNKS) - 1:
            cp_w(ci, 2).wait()
        gg = lax.dot_general(h2b, wg_buf[f0:f0 + fn, :], nt_dims, preferred_element_type=f32)
        uu = lax.dot_general(h2b, wu_buf[f0:f0 + fn, :], nt_dims, preferred_element_type=f32)
        act = (gg * jax.nn.sigmoid(gg) * uu).astype(bf16)
        acc = acc + jnp.dot(act, wd_buf[f0:f0 + fn, :], preferred_element_type=f32)
    o_sel = xc + mu + par[8, 0:1] * (h2 + acc * gate)

    row16d = lax.broadcasted_iota(jnp.int32, (16, D), 0)
    for t, idx in enumerate((i1, i2)):
        reg = idx // (S // NREG)
        step = (idx % (S // NREG)) // OROWS
        r16 = pl.ds(pl.multiple_of(((idx % OROWS) // 16) * 16, 16), 16)
        tile = o_buf[reg, step, r16, :].astype(f32)
        tile = jnp.where(row16d == idx % 16, o_sel[t:t + 1], tile)
        o_buf[reg, step, r16, :] = tile.astype(bf16)
    cp_out(lo).start()
    cp_out(hi).start()


def _kernel(*refs):
    pl.run_scoped(lambda sem: _body(*refs, sem), pltpu.SemaphoreType.DMA((N_IN_SEM,)))
    out_hbm, o_buf, sem_o = refs[13], refs[-5], refs[-1]
    pltpu.make_async_copy(o_buf, out_hbm, sem_o.at[0]).wait()


@jax.jit
def pallas_adaLN_cond__ssm_conv_h3__moe_arch_mod__prompt_kernel(
    A_q, A_k, A_v, A_shift_k, A_ssm_k, A_ssm_D, B_x, B_w_r, B_w_gate, B_w_up, B_w_down, c, w_mod,
):
    del B_x
    args = (
        A_q.reshape(S, D), A_k.reshape(S, D), A_v.reshape(S, D), A_shift_k.T, A_ssm_k,
        A_ssm_D.reshape(NT, 128), B_w_r.reshape(NT, 128), B_w_gate.T, B_w_up.T, B_w_down,
        c, w_mod, jnp.asarray(_dft_consts()),
    )
    vm = pltpu.VMEM
    in_bufs = [vm(a.shape, a.dtype) for a in args]
    in_bufs[1] = vm((HALO + S, D), bf16)
    scratch = in_bufs + [
        vm((NT, NG, 2, 8, 128), f32),
        vm((NT, NB, 3, NG, 8, 128), f32),
        vm((NB, 64, 128), u32),
        vm((NB, NG, 2, 8, 128), f32),
        vm((NB, NG, 2, 8, 128), f32),
        vm((NB, B, 128), u32),
        vm((NB, B, 128), u32),
        vm((NT, S, 128), f32),
        vm((NT, S, 128), f32),
        vm((NT, S, 128), f32),
        vm((NT, S, 128), f32),
        vm((NT, S, 128), f32),
        vm((S, 128), f32),
        vm((S, 128), f32),
        vm((S, 128), f32),
        vm((S, 128), f32),
        vm((S, 128), f32),
        vm((NREG, NB, OROWS, D), bf16),
        vm((9, 8, D), f32),
        vm((2, 8, 128), f32),
        pltpu.SMEM((4,), jnp.int32),
        pltpu.SemaphoreType.DMA((1,)),
    ]
    out = pl.pallas_call(
        _kernel,
        out_shape=jax.ShapeDtypeStruct((NREG, NB, OROWS, D), bf16),
        in_specs=[pl.BlockSpec(memory_space=pl.ANY)] * len(args),
        out_specs=pl.BlockSpec(memory_space=pl.ANY),
        scratch_shapes=scratch,
        compiler_params=pltpu.CompilerParams(vmem_limit_bytes=120 * 1024 * 1024),
        name="adaln_h3_mod",
    )(*args)
    return out.reshape(1, S, D)
```

```python
import math

import numpy as np
import jax
import jax.numpy as jnp
from jax import lax
import jax.experimental.pallas as pl
import jax.experimental.pallas.tpu as pltpu

S = 2048
D = 640
B = 128
NB = S // B
NT = D // 128
NG = B // 8
EPS = 1e-5
KV_CH = 256
NKV = S // KV_CH
HALO = 16
NREG = 4
OROWS = S // (NREG * NB)
GPI = 4
F_CHUNKS = ((0, 512), (512, 512), (1024, 384), (1408, 320))
N_IN_SEM = 5 + NT + 2 * NKV + 2 + 3 * len(F_CHUNKS)

f32 = jnp.float32
bf16 = jnp.bfloat16
u32 = jnp.uint32


def _dft_consts():
    k = np.concatenate([np.arange(0, B, 2), np.arange(1, B, 2)]).astype(np.float64)
    n = np.arange(B, dtype=np.float64)
    th = 2.0 * np.pi * (k[:, None] + 0.5) * n[None, :] / (2 * B)
    fwd = np.stack([np.cos(th).reshape(NG, 8, B), -np.sin(th).reshape(NG, 8, B)], axis=1).reshape(2 * B, B)
    n2 = np.arange(B, 2 * B, dtype=np.float64)
    th2 = 2.0 * np.pi * (k[None, :] + 0.5) * n2[:, None] / (2 * B)
    inv = np.stack([np.cos(th2).reshape(B, NG, 8), -np.sin(th2).reshape(B, NG, 8)], axis=2).reshape(B, 2 * B) / B
    inv = np.concatenate([inv[:, :B], inv[:, B:]], axis=0)
    mat = np.concatenate([fwd, inv], axis=0).astype(np.float32).astype(bf16)
    half = mat.view(np.uint16).astype(np.uint32)
    return half[0::2] | (half[1::2] << 16)


def _rs(ssq):
    return jnp.exp2(jnp.log(ssq + D * EPS) * (-0.5 / math.log(2.0)))


def _body(q_hbm, k_hbm, v_hbm, sk_hbm, h_hbm, dd_hbm, wr_hbm, wg_hbm, wu_hbm, wd_hbm,
          c_hbm, wm_hbm, fc_hbm,
          out_hbm,
          q_buf, k_buf, v_buf, sk_buf, h_buf, dd_buf, wr_buf, wg_buf, wu_buf, wd_buf,
          c_buf, wm_buf, fc_buf,
          prev, u_s, hp, g_a, g_b, y_a, y_b, y_lo, y_hi, xc_s, x2_s, xc2_s,
          st1, st2, st3, st4, st5, o_buf, par, r_s, zs,
          sem_o, sem):
    o_small, o_h, o_k, o_v, o_wm, o_q, o_w = [int(o) for o in np.cumsum([0, 5, NT, NKV, NKV, 1, 1])]
    small = [(fc_hbm, fc_buf), (sk_hbm, sk_buf), (dd_hbm, dd_buf), (c_hbm, c_buf), (wr_hbm, wr_buf)]
    cp_small = [pltpu.make_async_copy(s, d, sem.at[o_small + i]) for i, (s, d) in enumerate(small)]

    def cp_rows(src, dst, off, i, rows):
        return pltpu.make_async_copy(src.at[pl.ds(i * rows, rows)], dst.at[pl.ds(i * rows, rows)], sem.at[off + i])

    def cp_k(i):
        return pltpu.make_async_copy(k_hbm.at[pl.ds(i * KV_CH, KV_CH)],
                                     k_buf.at[pl.ds(HALO + i * KV_CH, KV_CH)], sem.at[o_k + i])

    def cp_h(j):
        return cp_rows(h_hbm, h_buf, o_h, j, 128)

    cp_wm = pltpu.make_async_copy(wm_hbm, wm_buf, sem.at[o_wm])
    cp_q = pltpu.make_async_copy(q_hbm, q_buf, sem.at[o_q])

    def cp_w(ci, t):
        f0, fn = F_CHUNKS[ci]
        src, dst = ((wg_hbm, wg_buf), (wu_hbm, wu_buf), (wd_hbm, wd_buf))[t]
        return pltpu.make_async_copy(src.at[pl.ds(f0, fn)], dst.at[pl.ds(f0, fn)], sem.at[o_w + ci * 3 + t])

    cp_small[0].start()
    cp_h(0).start()
    for c in cp_small[1:]:
        c.start()
    for i in range(NKV):
        cp_k(i).start()
        cp_rows(v_hbm, v_buf, o_v, i, KV_CH).start()
    for j in range(1, NT):
        cp_h(j).start()
    cp_wm.start()
    cp_q.start()
    for ci in range(len(F_CHUNKS)):
        for t in range(3):
            cp_w(ci, t).start()

    for t in range(4):
        zs[t] = 0
    for j in range(NT):
        prev[j] = jnp.zeros((NG, 2, 8, 128), f32)
    r_s[...] = jnp.zeros((2, 8, 128), f32)
    k_buf[0:HALO, :] = jnp.zeros((HALO, D), bf16)

    nt_dims = (((1,), (1,)), ((), ()))
    inv_d = 1.0 / D

    def as_bf16(w):
        return pltpu.bitcast(w, bf16)

    def f_fwd():
        return as_bf16(fc_buf[0:B, :])

    def h_tile(j, m):
        return h_buf[pl.ds(j * 128, 128), pl.ds(pl.multiple_of(m * B, B), B)]

    def stage_r(j, m):
        hp[m] = pltpu.bitcast(h_tile(j, m), u32)

    def stage_h(tile, m, g_dst):
        hh = lax.dot_general(f_fwd(), tile, nt_dims, preferred_element_type=f32)
        g_dst[m] = hh.reshape(NG, 2, 8, 128)

    def fix_d(j, g_dst):
        dj = dd_buf[j:j + 1, :].astype(f32)[None]
        g_dst[0, :, 0] = g_dst[0, :, 0] + dj

    def stage_i(j, a, y_src):
        rows = pl.ds(pl.multiple_of(a * B, B), B)
        hb = B // 2
        y_lo[j, rows, :] = jnp.dot(as_bf16(fc_buf[B:B + hb, :]), as_bf16(y_src[a, 0:hb]),
                                   preferred_element_type=f32)
        y_hi[j, rows, :] = jnp.dot(as_bf16(fc_buf[B + hb:, :]), as_bf16(y_src[a, hb:]),
                                   preferred_element_type=f32)

    def stage_c(j, g, g_src, y_dst):
        for half in range(2):
            gg = jnp.clip(g + zs[half], 0, NG - 1)
            g2 = jnp.clip(g + zs[2 + half], 0, NG - 1)
            lo = half * 8
            n_in = lo + 8
            res = []
            for comp in range(3):
                acc = [None] * 8 if comp == 0 else list(res[0])
                v = {}
                for jj in range(n_in):
                    u = u_s[j, jj, comp, gg]
                    for o in range(8):
                        m = lo + o - jj
                        if m < 0:
                            continue
                        if m not in v:
                            if comp == 0:
                                v[m] = g_src[m, g2, 0] + g_src[m, g2, 1]
                            else:
                                v[m] = g_src[m, gg, comp - 1]
                        p = u * v[m]
                        if acc[o] is None:
                            acc[o] = p
                        elif comp == 2:
                            acc[o] = acc[o] - p
                        else:
                            acc[o] = acc[o] + p
                res.append(acc)
                if comp > 0:
                    r4 = pl.ds(pl.multiple_of(g * 8 + 4 * (2 - comp), 4), 4)
                    for o in range(8):
                        y_dst[lo + o, r4, :] = pltpu.bitcast(acc[o].astype(bf16), u32)

    def lanes(t):
        return slice(t * 128, (t + 1) * 128)

    def rsum(xs):
        s = xs[0]
        for x in xs[1:]:
            s = s + x
        return jnp.broadcast_to(jnp.sum(s, axis=1, keepdims=True), (8, 128))

    def grp(r0, gi):
        return pl.ds(pl.multiple_of(r0 + gi * 8, 8), 8)

    def stage_a(r0, nrows):
        for gi in range(nrows // 8):
            rows = grp(r0, gi)
            st1[rows, :] = rsum([q_buf[rows, lanes(t)].astype(f32) for t in range(NT)]) * inv_d

    def stage_b(r0, nrows):
        for gi in range(nrows // 8):
            rows = grp(r0, gi)
            mu = st1[rows, :]
            sq = []
            for t in range(NT):
                xc = q_buf[rows, lanes(t)].astype(f32) - mu
                xc_s[t, rows, :] = xc
                sq.append(xc * xc)
            st2[rows, :] = _rs(rsum(sq))

    def stage_x(r0):
        for gi in range(NG):
            rows = grp(r0, gi)
            rs = st2[rows, :]
            xs = []
            for t in range(NT):
                xc = xc_s[t, rows, :]
                y = y_lo[t, rows, :] + y_hi[t, rows, :]
                x2 = ((xc * rs) * par[0, :, lanes(t)] + par[1, :, lanes(t)]) * y + xc
                x2_s[t, rows, :] = x2
                xs.append(x2)
            st3[rows, :] = rsum(xs) * inv_d

    def stage_d(r0):
        for gi in range(NG):
            rows = grp(r0, gi)
            mu = st3[rows, :]
            sq, rd = [], []
            for t in range(NT):
                xc = x2_s[t, rows, :] - mu
                xc2_s[t, rows, :] = xc
                sq.append(xc * xc)
                rd.append(xc * par[4, :, lanes(t)])
            rs = _rs(rsum(sq))
            st4[rows, :] = rs
            st5[rows, :] = rsum(rd) * rs

    lane = lax.broadcasted_iota(jnp.int32, (8, 128), 1)

    def stage_e(a, r0):
        rblk = r_s[a // 8]
        lane_rel = lane - (a % 8) * NG
        for gi in range(NG):
            rows = grp(r0, gi)
            rs = st4[rows, :]
            mu = st1[rows, :] + st3[rows, :]
            rblk = jnp.where(lane_rel == gi, st5[rows, :], rblk)
            for t in range(NT):
                xc = xc2_s[t, rows, :]
                out = (xc * rs) * par[2, :, lanes(t)] + xc + (par[3, :, lanes(t)] + mu)
                o_buf[a // NREG, (a % NREG) * NREG + gi // 4, (gi % 4) * 8:(gi % 4) * 8 + 8, lanes(t)] = (
                    out.astype(bf16))
        r_s[a // 8] = rblk

    def build_par():
        cf = c_buf[...].astype(f32)
        cs = (cf * jax.nn.sigmoid(cf)).astype(bf16)
        mod = jnp.dot(jnp.broadcast_to(cs, (16, D)), wm_buf[...], preferred_element_type=f32)[0:8]
        sa, ca, ga, sb, cb, gb = [mod[:, i * D:(i + 1) * D] for i in range(6)]
        wr = jnp.concatenate([jnp.broadcast_to(wr_buf[t:t + 1, :].astype(f32), (8, 128))
                              for t in range(NT)], axis=1)
        sqd = math.sqrt(D)
        par[0] = ga * (1.0 + ca) * sqd
        par[1] = ga * sa
        par[2] = gb * (1.0 + cb) * sqd
        par[3] = gb * sb
        par[4] = (1.0 + cb) * wr
        par[5] = wr
        par[6] = (1.0 + cb) * sqd
        par[7] = sb
        par[8] = gb

    cp_small[0].wait()
    cp_h(0).wait()

    for m in range(NB):
        stage_h(h_tile(0, m), m, g_a)
    for c in cp_small[1:]:
        c.wait()
    fix_d(0, g_a)

    def p_body(i, c):
        cp_k(i).wait()
        cp_rows(v_hbm, v_buf, o_v, i, KV_CH).wait()
        sk = sk_buf[...].astype(f32)
        nblk = KV_CH // B
        for j in range(NT):
            ls = lanes(j)
            for t in range(nblk):
                a = i * nblk + t
                r0 = pl.multiple_of(a * B, B)
                kw = k_buf[pl.ds(r0 + HALO - 8, B + 8), ls].astype(f32)
                ks = kw[8:] * sk[0:1, ls]
                for t2 in range(1, 4):
                    ks = ks + kw[8 - t2:B + 8 - t2] * sk[t2:t2 + 1, ls]
                kv = (ks * v_buf[pl.ds(r0, B), ls].astype(f32)).astype(bf16)
                x = jnp.dot(f_fwd(), kv, preferred_element_type=f32).reshape(NG, 2, 8, 128)
                p = prev[j] if t == 0 else xprev
                xprev = x
                if t == nblk - 1:
                    prev[j] = x
                hb = NG // 2
                wr_ = jnp.concatenate([p[:hb, 0] + x[:hb, 1], p[hb:, 0] - x[hb:, 1]], axis=0)
                wi_ = jnp.concatenate([p[:hb, 1] - x[:hb, 0], p[hb:, 1] + x[hb:, 0]], axis=0)
                u_s[j, a, 0] = wr_
                u_s[j, a, 1] = wi_ - wr_
                u_s[j, a, 2] = wr_ + wi_
        return c
    lax.fori_loop(0, NKV, p_body, 0)

    gs = (g_a, g_b)
    ys = (y_a, y_b)
    n_it = NG // GPI
    for j in range(NT):
        if j + 1 < NT:
            cp_h(j + 1).wait()
            for m in range(NB):
                stage_r(j + 1, m)

        def c_body(i, c, j=j):
            for t in range(GPI):
                g = i * GPI + t
                if j + 1 < NT:
                    stage_h(as_bf16(hp[g]), g, gs[(j + 1) % 2])
                if j > 0:
                    stage_i(j - 1, g, ys[(j - 1) % 2])
                stage_c(j, g, gs[j % 2], ys[j % 2])
            return c
        lax.fori_loop(0, n_it, c_body, 0)
        if j + 1 < NT:
            fix_d(j + 1, gs[(j + 1) % 2])

    y_last = ys[(NT - 1) % 2]
    cp_wm.wait()
    cp_q.wait()
    build_par()
    for a in range(3):
        stage_i(NT - 1, a, y_last)
    stage_a(0, S)
    stage_b(0, S)
    stage_x(0)
    stage_x(B)
    stage_d(0)

    def e_body(a, c):
        stage_i(NT - 1, a + 3, y_last)
        stage_x((a + 2) * B)
        stage_d((a + 1) * B)
        stage_e(a, a * B)
        return c
    lax.fori_loop(0, NB - 3, e_body, 0)
    stage_x((NB - 1) * B)
    stage_d((NB - 2) * B)
    stage_e(NB - 3, (NB - 3) * B)
    stage_d((NB - 1) * B)
    stage_e(NB - 2, (NB - 2) * B)
    stage_e(NB - 1, (NB - 1) * B)

    rall = r_s[...].reshape(16, 128)
    sub = lax.broadcasted_iota(jnp.int32, (16, 128), 0)
    ln = lax.broadcasted_iota(jnp.int32, (16, 128), 1)
    ridx = (sub // 8) * (S // 2) + ln * 8 + (sub % 8)
    bits = lax.bitcast_convert_type(rall, jnp.int32)
    bits = jnp.where((bits & jnp.int32(0x7F800000)) == 0, jnp.int32(0x00800000), bits)
    code = jnp.where(bits < 0, ridx, S - 1 - ridx)
    key = lax.bitcast_convert_type((bits & jnp.int32(-S)) | code, f32)
    m1 = jnp.max(key, axis=1, keepdims=True)
    m2 = jnp.max(jnp.where(key == m1, -jnp.inf, key), axis=1, keepdims=True)
    g1 = jnp.max(m1, axis=0, keepdims=True)
    g2 = jnp.max(jnp.where(m1 == g1, m2, m1), axis=0, keepdims=True)

    def decode(g):
        gb = lax.bitcast_convert_type(g, jnp.int32)
        c = gb & (S - 1)
        return jnp.clip(jnp.where(gb < 0, c, S - 1 - c)[0, 0], 0, S - 1)

    i1 = decode(g1)
    i2 = decode(g2)

    c1 = (i1 % (S // NREG)) // OROWS
    c2 = (i2 % (S // NREG)) // OROWS
    c2 = jnp.where(c1 == c2, (c1 + 1) % NB, c2)
    lo = jnp.minimum(c1, c2)
    hi = jnp.maximum(c1, c2)

    def cp_out(blk):
        return pltpu.make_async_copy(o_buf.at[:, blk], out_hbm.at[:, blk], sem_o.at[0])

    def early_blk(s):
        o = s + (s >= lo).astype(jnp.int32)
        return o + (o >= hi).astype(jnp.int32)

    for ci in range(len(F_CHUNKS)):
        for t in range(3):
            if (ci, t) != (len(F_CHUNKS) - 1, 2):
                cp_w(ci, t).wait()
    for s in range(NB - 2):
        cp_out(early_blk(s)).start()

    row16 = lax.broadcasted_iota(jnp.int32, (16, 128), 0)

    def pick(ref_rows):
        return jnp.where(row16 == 0, ref_rows(i1), jnp.where(row16 == 1, ref_rows(i2), 0.0))

    xc = jnp.concatenate([pick(lambda i, t=t: xc2_s[t, pl.ds(i, 1), :]) for t in range(NT)], axis=1)
    rs = pick(lambda i: st4[pl.ds(i, 1), :])[:, 0:1]
    mu = pick(lambda i: st1[pl.ds(i, 1), :] + st3[pl.ds(i, 1), :])[:, 0:1]
    h2 = xc * rs * par[6, 0:1] + par[7, 0:1]
    gate = jax.nn.sigmoid(jnp.sum(h2 * par[5, 0:1], axis=1, keepdims=True))
    h2b = h2.astype(bf16)

    acc = jnp.zeros((16, D), f32)
    for ci, (f0, fn) in enumerate(F_CHUNKS):
        if ci == len(F_CHUNKS) - 1:
            cp_w(ci, 2).wait()
        gg = lax.dot_general(h2b, wg_buf[f0:f0 + fn, :], nt_dims, preferred_element_type=f32)
        uu = lax.dot_general(h2b, wu_buf[f0:f0 + fn, :], nt_dims, preferred_element_type=f32)
        act = (gg * jax.nn.sigmoid(gg) * uu).astype(bf16)
        acc = acc + jnp.dot(act, wd_buf[f0:f0 + fn, :], preferred_element_type=f32)
    o_sel = xc + mu + par[8, 0:1] * (h2 + acc * gate)

    row16d = lax.broadcasted_iota(jnp.int32, (16, D), 0)
    for t, idx in enumerate((i1, i2)):
        reg = idx // (S // NREG)
        step = (idx % (S // NREG)) // OROWS
        r16 = pl.ds(pl.multiple_of(((idx % OROWS) // 16) * 16, 16), 16)
        tile = o_buf[reg, step, r16, :].astype(f32)
        tile = jnp.where(row16d == idx % 16, o_sel[t:t + 1], tile)
        o_buf[reg, step, r16, :] = tile.astype(bf16)
    cp_out(lo).start()
    cp_out(hi).start()


def _kernel(*refs):
    pl.run_scoped(lambda sem: _body(*refs, sem), pltpu.SemaphoreType.DMA((N_IN_SEM,)))
    out_hbm, o_buf, sem_o = refs[13], refs[-5], refs[-1]
    pltpu.make_async_copy(o_buf, out_hbm, sem_o.at[0]).wait()


@jax.jit
def pallas_adaLN_cond__ssm_conv_h3__moe_arch_mod__prompt_kernel(
    A_q, A_k, A_v, A_shift_k, A_ssm_k, A_ssm_D, B_x, B_w_r, B_w_gate, B_w_up, B_w_down, c, w_mod,
):
    del B_x
    args = (
        A_q.reshape(S, D), A_k.reshape(S, D), A_v.reshape(S, D), A_shift_k.T, A_ssm_k,
        A_ssm_D.reshape(NT, 128), B_w_r.reshape(NT, 128), B_w_gate.T, B_w_up.T, B_w_down,
        c, w_mod, jnp.asarray(_dft_consts()),
    )
    vm = pltpu.VMEM
    in_bufs = [vm(a.shape, a.dtype) for a in args]
    in_bufs[1] = vm((HALO + S, D), bf16)
    scratch = in_bufs + [
        vm((NT, NG, 2, 8, 128), f32),
        vm((NT, NB, 3, NG, 8, 128), f32),
        vm((NB, 64, 128), u32),
        vm((NB, NG, 2, 8, 128), f32),
        vm((NB, NG, 2, 8, 128), f32),
        vm((NB, B, 128), u32),
        vm((NB, B, 128), u32),
        vm((NT, S, 128), f32),
        vm((NT, S, 128), f32),
        vm((NT, S, 128), f32),
        vm((NT, S, 128), f32),
        vm((NT, S, 128), f32),
        vm((S, 128), f32),
        vm((S, 128), f32),
        vm((S, 128), f32),
        vm((S, 128), f32),
        vm((S, 128), f32),
        vm((NREG, NB, OROWS, D), bf16),
        vm((9, 8, D), f32),
        vm((2, 8, 128), f32),
        pltpu.SMEM((4,), jnp.int32),
        pltpu.SemaphoreType.DMA((1,)),
    ]
    out = pl.pallas_call(
        _kernel,
        out_shape=jax.ShapeDtypeStruct((NREG, NB, OROWS, D), bf16),
        in_specs=[pl.BlockSpec(memory_space=pl.ANY)] * len(args),
        out_specs=pl.BlockSpec(memory_space=pl.ANY),
        scratch_shapes=scratch,
        compiler_params=pltpu.CompilerParams(vmem_limit_bytes=120 * 1024 * 1024),
        name="adaln_h3_mod",
    )(*args)
    return out.reshape(1, S, D)
```

```python
import math

import numpy as np
import jax
import jax.numpy as jnp
from jax import lax
import jax.experimental.pallas as pl
import jax.experimental.pallas.tpu as pltpu

S = 2048
D = 640
B = 128
NB = S // B
NT = D // 128
NG = B // 8
EPS = 1e-5
KV_CH = 256
NKV = S // KV_CH
HALO = 16
NREG = 4
OROWS = S // (NREG * NB)
GPI = 4
F_CHUNKS = ((0, 512), (512, 512), (1024, 384), (1408, 320))
N_IN_SEM = 4 + NT + 2 * NKV + 2 + 3 * len(F_CHUNKS)

f32 = jnp.float32
bf16 = jnp.bfloat16
u32 = jnp.uint32


def _dft_operands():
    r = lax.broadcasted_iota(jnp.int32, (8, B), 0)
    n = lax.broadcasted_iota(jnp.int32, (8, B), 1)
    ang = jnp.concatenate([(4 * r + 1) * n, (4 * r + 3) * n, 32 * n], axis=0)
    ang = jnp.concatenate([ang, ang + B], axis=0) & (4 * B - 1)
    seed = jnp.cos(ang.astype(f32) * (2.0 * math.pi / (4 * B)))
    cs, ms = seed[16:24], seed[40:48]
    fwd, inv = [], []
    for odd in range(2):
        c, m = seed[8 * odd:8 * odd + 8], seed[24 + 8 * odd:32 + 8 * odd]
        sgn = (-1.0 if odd else 1.0) / B
        for gi in range(NG // 2):
            if gi:
                c, m = c * cs - m * ms, m * cs + c * ms
            fwd += [c, m]
            inv += [m * sgn, c * (-sgn)]
    fwd = jnp.concatenate(fwd, axis=0)
    inv = [jnp.concatenate(inv[NG * hh:NG * (hh + 1)], axis=0).T for hh in range(2)]
    return pltpu.bitcast(jnp.concatenate([fwd] + inv, axis=0).astype(bf16), u32)


def _rs(ssq):
    return jnp.exp2(jnp.log(ssq + D * EPS) * (-0.5 / math.log(2.0)))


def _body(q_hbm, k_hbm, v_hbm, sk_hbm, h_hbm, dd_hbm, wr_hbm, wg_hbm, wu_hbm, wd_hbm,
          c_hbm, wm_hbm,
          out_hbm,
          q_buf, k_buf, v_buf, sk_buf, h_buf, dd_buf, wr_buf, wg_buf, wu_buf, wd_buf,
          c_buf, wm_buf,
          fc_buf, prev, u_s, hp, g_a, g_b, y_a, y_b, y_lo, y_hi, xc_s, x2_s, xc2_s,
          st1, st2, st3, st4, st5, o_buf, par, r_s, zs,
          sem_o, sem):
    o_small, o_h, o_k, o_v, o_wm, o_q, o_w = [int(o) for o in np.cumsum([0, 4, NT, NKV, NKV, 1, 1])]
    small = [(sk_hbm, sk_buf), (dd_hbm, dd_buf), (c_hbm, c_buf), (wr_hbm, wr_buf)]
    cp_small = [pltpu.make_async_copy(s, d, sem.at[o_small + i]) for i, (s, d) in enumerate(small)]

    def cp_rows(src, dst, off, i, rows):
        return pltpu.make_async_copy(src.at[pl.ds(i * rows, rows)], dst.at[pl.ds(i * rows, rows)], sem.at[off + i])

    def cp_k(i):
        return pltpu.make_async_copy(k_hbm.at[pl.ds(i * KV_CH, KV_CH)],
                                     k_buf.at[pl.ds(HALO + i * KV_CH, KV_CH)], sem.at[o_k + i])

    def cp_h(j):
        return cp_rows(h_hbm, h_buf, o_h, j, 128)

    cp_wm = pltpu.make_async_copy(wm_hbm, wm_buf, sem.at[o_wm])
    cp_q = pltpu.make_async_copy(q_hbm, q_buf, sem.at[o_q])

    def cp_w(ci, t):
        f0, fn = F_CHUNKS[ci]
        src, dst = ((wg_hbm, wg_buf), (wu_hbm, wu_buf), (wd_hbm, wd_buf))[t]
        return pltpu.make_async_copy(src.at[pl.ds(f0, fn)], dst.at[pl.ds(f0, fn)], sem.at[o_w + ci * 3 + t])

    cp_h(0).start()
    for c in cp_small:
        c.start()
    for i in range(NKV):
        cp_k(i).start()
        cp_rows(v_hbm, v_buf, o_v, i, KV_CH).start()
    for j in range(1, NT):
        cp_h(j).start()
    cp_wm.start()
    cp_q.start()
    for ci in range(len(F_CHUNKS)):
        for t in range(3):
            cp_w(ci, t).start()

    for t in range(4):
        zs[t] = 0
    for j in range(NT):
        prev[j] = jnp.zeros((NG, 2, 8, 128), f32)
    r_s[...] = jnp.zeros((2, 8, 128), f32)
    k_buf[0:HALO, :] = jnp.zeros((HALO, D), bf16)
    fc_buf[...] = _dft_operands()

    nt_dims = (((1,), (1,)), ((), ()))
    inv_d = 1.0 / D

    def as_bf16(w):
        return pltpu.bitcast(w, bf16)

    def f_fwd():
        return as_bf16(fc_buf[0:B, :])

    def h_tile(j, m):
        return h_buf[pl.ds(j * 128, 128), pl.ds(pl.multiple_of(m * B, B), B)]

    def stage_r(j, m):
        hp[m] = pltpu.bitcast(h_tile(j, m), u32)

    def stage_h(tile, m, g_dst):
        hh = lax.dot_general(f_fwd(), tile, nt_dims, preferred_element_type=f32)
        g_dst[m] = hh.reshape(NG, 2, 8, 128)

    def fix_d(j, g_dst):
        dj = dd_buf[j:j + 1, :].astype(f32)[None]
        g_dst[0, :, 0] = g_dst[0, :, 0] + dj

    def stage_i(j, a, y_src):
        rows = pl.ds(pl.multiple_of(a * B, B), B)
        hb = B // 2
        y_lo[j, rows, :] = jnp.dot(as_bf16(fc_buf[B:B + hb, :]), as_bf16(y_src[a, 0:hb]),
                                   preferred_element_type=f32)
        y_hi[j, rows, :] = jnp.dot(as_bf16(fc_buf[B + hb:, :]), as_bf16(y_src[a, hb:]),
                                   preferred_element_type=f32)

    def stage_c(j, g, g_src, y_dst):
        for half in range(2):
            gg = jnp.clip(g + zs[half], 0, NG - 1)
            g2 = jnp.clip(g + zs[2 + half], 0, NG - 1)
            lo = half * 8
            n_in = lo + 8
            res = []
            for comp in range(3):
                acc = [None] * 8 if comp == 0 else list(res[0])
                v = {}
                for jj in range(n_in):
                    u = u_s[j, jj, comp, gg]
                    for o in range(8):
                        m = lo + o - jj
                        if m < 0:
                            continue
                        if m not in v:
                            if comp == 0:
                                v[m] = g_src[m, g2, 0] + g_src[m, g2, 1]
                            else:
                                v[m] = g_src[m, gg, comp - 1]
                        p = u * v[m]
                        if acc[o] is None:
                            acc[o] = p
                        elif comp == 2:
                            acc[o] = acc[o] - p
                        else:
                            acc[o] = acc[o] + p
                res.append(acc)
                if comp > 0:
                    r4 = pl.ds(pl.multiple_of(g * 8 + 4 * (2 - comp), 4), 4)
                    for o in range(8):
                        y_dst[lo + o, r4, :] = pltpu.bitcast(acc[o].astype(bf16), u32)

    def lanes(t):
        return slice(t * 128, (t + 1) * 128)

    def rsum(xs):
        s = xs[0]
        for x in xs[1:]:
            s = s + x
        return jnp.broadcast_to(jnp.sum(s, axis=1, keepdims=True), (8, 128))

    def grp(r0, gi):
        return pl.ds(pl.multiple_of(r0 + gi * 8, 8), 8)

    def stage_a(r0, nrows):
        for gi in range(nrows // 8):
            rows = grp(r0, gi)
            st1[rows, :] = rsum([q_buf[rows, lanes(t)].astype(f32) for t in range(NT)]) * inv_d

    def stage_b(r0, nrows):
        for gi in range(nrows // 8):
            rows = grp(r0, gi)
            mu = st1[rows, :]
            sq = []
            for t in range(NT):
                xc = q_buf[rows, lanes(t)].astype(f32) - mu
                xc_s[t, rows, :] = xc
                sq.append(xc * xc)
            st2[rows, :] = _rs(rsum(sq))

    def stage_x(r0):
        for gi in range(NG):
            rows = grp(r0, gi)
            rs = st2[rows, :]
            xs = []
            for t in range(NT):
                xc = xc_s[t, rows, :]
                y = y_lo[t, rows, :] + y_hi[t, rows, :]
                x2 = ((xc * rs) * par[0, :, lanes(t)] + par[1, :, lanes(t)]) * y + xc
                x2_s[t, rows, :] = x2
                xs.append(x2)
            st3[rows, :] = rsum(xs) * inv_d

    def stage_d(r0):
        for gi in range(NG):
            rows = grp(r0, gi)
            mu = st3[rows, :]
            sq, rd = [], []
            for t in range(NT):
                xc = x2_s[t, rows, :] - mu
                xc2_s[t, rows, :] = xc
                sq.append(xc * xc)
                rd.append(xc * par[4, :, lanes(t)])
            rs = _rs(rsum(sq))
            st4[rows, :] = rs
            st5[rows, :] = rsum(rd) * rs

    lane = lax.broadcasted_iota(jnp.int32, (8, 128), 1)

    def stage_e(a, r0):
        rblk = r_s[a // 8]
        lane_rel = lane - (a % 8) * NG
        for gi in range(NG):
            rows = grp(r0, gi)
            rs = st4[rows, :]
            mu = st1[rows, :] + st3[rows, :]
            rblk = jnp.where(lane_rel == gi, st5[rows, :], rblk)
            for t in range(NT):
                xc = xc2_s[t, rows, :]
                out = (xc * rs) * par[2, :, lanes(t)] + xc + (par[3, :, lanes(t)] + mu)
                o_buf[a // NREG, (a % NREG) * NREG + gi // 4, (gi % 4) * 8:(gi % 4) * 8 + 8, lanes(t)] = (
                    out.astype(bf16))
        r_s[a // 8] = rblk

    def build_par():
        cf = c_buf[...].astype(f32)
        cs = (cf * jax.nn.sigmoid(cf)).astype(bf16)
        mod = jnp.dot(jnp.broadcast_to(cs, (16, D)), wm_buf[...], preferred_element_type=f32)[0:8]
        sa, ca, ga, sb, cb, gb = [mod[:, i * D:(i + 1) * D] for i in range(6)]
        wr = jnp.concatenate([jnp.broadcast_to(wr_buf[t:t + 1, :].astype(f32), (8, 128))
                              for t in range(NT)], axis=1)
        sqd = math.sqrt(D)
        par[0] = ga * (1.0 + ca) * sqd
        par[1] = ga * sa
        par[2] = gb * (1.0 + cb) * sqd
        par[3] = gb * sb
        par[4] = (1.0 + cb) * wr
        par[5] = wr
        par[6] = (1.0 + cb) * sqd
        par[7] = sb
        par[8] = gb

    cp_h(0).wait()

    for m in range(NB):
        stage_h(h_tile(0, m), m, g_a)
    for c in cp_small:
        c.wait()
    fix_d(0, g_a)

    def p_body(i, c):
        cp_k(i).wait()
        cp_rows(v_hbm, v_buf, o_v, i, KV_CH).wait()
        sk = sk_buf[...].astype(f32)
        nblk = KV_CH // B
        for j in range(NT):
            ls = lanes(j)
            for t in range(nblk):
                a = i * nblk + t
                r0 = pl.multiple_of(a * B, B)
                kw = k_buf[pl.ds(r0 + HALO - 8, B + 8), ls].astype(f32)
                ks = kw[8:] * sk[0:1, ls]
                for t2 in range(1, 4):
                    ks = ks + kw[8 - t2:B + 8 - t2] * sk[t2:t2 + 1, ls]
                kv = (ks * v_buf[pl.ds(r0, B), ls].astype(f32)).astype(bf16)
                x = jnp.dot(f_fwd(), kv, preferred_element_type=f32).reshape(NG, 2, 8, 128)
                p = prev[j] if t == 0 else xprev
                xprev = x
                if t == nblk - 1:
                    prev[j] = x
                hb = NG // 2
                wr_ = jnp.concatenate([p[:hb, 0] + x[:hb, 1], p[hb:, 0] - x[hb:, 1]], axis=0)
                wi_ = jnp.concatenate([p[:hb, 1] - x[:hb, 0], p[hb:, 1] + x[hb:, 0]], axis=0)
                u_s[j, a, 0] = wr_
                u_s[j, a, 1] = wi_ - wr_
                u_s[j, a, 2] = wr_ + wi_
        return c
    lax.fori_loop(0, NKV, p_body, 0)

    gs = (g_a, g_b)
    ys = (y_a, y_b)
    n_it = NG // GPI
    for j in range(NT):
        if j + 1 < NT:
            cp_h(j + 1).wait()
            for m in range(NB):
                stage_r(j + 1, m)

        def c_body(i, c, j=j):
            for t in range(GPI):
                g = i * GPI + t
                if j + 1 < NT:
                    stage_h(as_bf16(hp[g]), g, gs[(j + 1) % 2])
                if j > 0:
                    stage_i(j - 1, g, ys[(j - 1) % 2])
                stage_c(j, g, gs[j % 2], ys[j % 2])
            return c
        lax.fori_loop(0, n_it, c_body, 0)
        if j + 1 < NT:
            fix_d(j + 1, gs[(j + 1) % 2])

    y_last = ys[(NT - 1) % 2]
    cp_wm.wait()
    cp_q.wait()
    build_par()
    for a in range(3):
        stage_i(NT - 1, a, y_last)
    stage_a(0, S)
    stage_b(0, S)
    stage_x(0)
    stage_x(B)
    stage_d(0)

    def e_body(a, c):
        stage_i(NT - 1, a + 3, y_last)
        stage_x((a + 2) * B)
        stage_d((a + 1) * B)
        stage_e(a, a * B)
        return c
    lax.fori_loop(0, NB - 3, e_body, 0)
    stage_x((NB - 1) * B)
    stage_d((NB - 2) * B)
    stage_e(NB - 3, (NB - 3) * B)
    stage_d((NB - 1) * B)
    stage_e(NB - 2, (NB - 2) * B)
    stage_e(NB - 1, (NB - 1) * B)

    rall = r_s[...].reshape(16, 128)
    sub = lax.broadcasted_iota(jnp.int32, (16, 128), 0)
    ln = lax.broadcasted_iota(jnp.int32, (16, 128), 1)
    ridx = (sub // 8) * (S // 2) + ln * 8 + (sub % 8)
    bits = lax.bitcast_convert_type(rall, jnp.int32)
    bits = jnp.where((bits & jnp.int32(0x7F800000)) == 0, jnp.int32(0x00800000), bits)
    code = jnp.where(bits < 0, ridx, S - 1 - ridx)
    key = lax.bitcast_convert_type((bits & jnp.int32(-S)) | code, f32)
    m1 = jnp.max(key, axis=1, keepdims=True)
    m2 = jnp.max(jnp.where(key == m1, -jnp.inf, key), axis=1, keepdims=True)
    g1 = jnp.max(m1, axis=0, keepdims=True)
    g2 = jnp.max(jnp.where(m1 == g1, m2, m1), axis=0, keepdims=True)

    def decode(g):
        gb = lax.bitcast_convert_type(g, jnp.int32)
        c = gb & (S - 1)
        return jnp.clip(jnp.where(gb < 0, c, S - 1 - c)[0, 0], 0, S - 1)

    i1 = decode(g1)
    i2 = decode(g2)

    c1 = (i1 % (S // NREG)) // OROWS
    c2 = (i2 % (S // NREG)) // OROWS
    c2 = jnp.where(c1 == c2, (c1 + 1) % NB, c2)
    lo = jnp.minimum(c1, c2)
    hi = jnp.maximum(c1, c2)

    def cp_out(blk):
        return pltpu.make_async_copy(o_buf.at[:, blk], out_hbm.at[:, blk], sem_o.at[0])

    def early_blk(s):
        o = s + (s >= lo).astype(jnp.int32)
        return o + (o >= hi).astype(jnp.int32)

    for ci in range(len(F_CHUNKS)):
        for t in range(3):
            if (ci, t) != (len(F_CHUNKS) - 1, 2):
                cp_w(ci, t).wait()
    for s in range(NB - 2):
        cp_out(early_blk(s)).start()

    row16 = lax.broadcasted_iota(jnp.int32, (16, 128), 0)

    def pick(ref_rows):
        return jnp.where(row16 == 0, ref_rows(i1), jnp.where(row16 == 1, ref_rows(i2), 0.0))

    xc = jnp.concatenate([pick(lambda i, t=t: xc2_s[t, pl.ds(i, 1), :]) for t in range(NT)], axis=1)
    rs = pick(lambda i: st4[pl.ds(i, 1), :])[:, 0:1]
    mu = pick(lambda i: st1[pl.ds(i, 1), :] + st3[pl.ds(i, 1), :])[:, 0:1]
    h2 = xc * rs * par[6, 0:1] + par[7, 0:1]
    gate = jax.nn.sigmoid(jnp.sum(h2 * par[5, 0:1], axis=1, keepdims=True))
    h2b = h2.astype(bf16)

    acc = jnp.zeros((16, D), f32)
    for ci, (f0, fn) in enumerate(F_CHUNKS):
        if ci == len(F_CHUNKS) - 1:
            cp_w(ci, 2).wait()
        gg = lax.dot_general(h2b, wg_buf[f0:f0 + fn, :], nt_dims, preferred_element_type=f32)
        uu = lax.dot_general(h2b, wu_buf[f0:f0 + fn, :], nt_dims, preferred_element_type=f32)
        act = (gg * jax.nn.sigmoid(gg) * uu).astype(bf16)
        acc = acc + jnp.dot(act, wd_buf[f0:f0 + fn, :], preferred_element_type=f32)
    o_sel = xc + mu + par[8, 0:1] * (h2 + acc * gate)

    row16d = lax.broadcasted_iota(jnp.int32, (16, D), 0)
    for t, idx in enumerate((i1, i2)):
        reg = idx // (S // NREG)
        step = (idx % (S // NREG)) // OROWS
        r16 = pl.ds(pl.multiple_of(((idx % OROWS) // 16) * 16, 16), 16)
        tile = o_buf[reg, step, r16, :].astype(f32)
        tile = jnp.where(row16d == idx % 16, o_sel[t:t + 1], tile)
        o_buf[reg, step, r16, :] = tile.astype(bf16)
    cp_out(lo).start()
    cp_out(hi).start()


def _kernel(*refs):
    pl.run_scoped(lambda sem: _body(*refs, sem), pltpu.SemaphoreType.DMA((N_IN_SEM,)))
    out_hbm, o_buf, sem_o = refs[12], refs[-5], refs[-1]
    pltpu.make_async_copy(o_buf, out_hbm, sem_o.at[0]).wait()


@jax.jit
def pallas_adaLN_cond__ssm_conv_h3__moe_arch_mod__prompt_kernel(
    A_q, A_k, A_v, A_shift_k, A_ssm_k, A_ssm_D, B_x, B_w_r, B_w_gate, B_w_up, B_w_down, c, w_mod,
):
    del B_x
    args = (
        A_q.reshape(S, D), A_k.reshape(S, D), A_v.reshape(S, D), A_shift_k.T, A_ssm_k,
        A_ssm_D.reshape(NT, 128), B_w_r.reshape(NT, 128), B_w_gate.T, B_w_up.T, B_w_down,
        c, w_mod,
    )
    vm = pltpu.VMEM
    in_bufs = [vm(a.shape, a.dtype) for a in args]
    in_bufs[1] = vm((HALO + S, D), bf16)
    scratch = in_bufs + [
        vm((2 * B, B), u32),
        vm((NT, NG, 2, 8, 128), f32),
        vm((NT, NB, 3, NG, 8, 128), f32),
        vm((NB, 64, 128), u32),
        vm((NB, NG, 2, 8, 128), f32),
        vm((NB, NG, 2, 8, 128), f32),
        vm((NB, B, 128), u32),
        vm((NB, B, 128), u32),
        vm((NT, S, 128), f32),
        vm((NT, S, 128), f32),
        vm((NT, S, 128), f32),
        vm((NT, S, 128), f32),
        vm((NT, S, 128), f32),
        vm((S, 128), f32),
        vm((S, 128), f32),
        vm((S, 128), f32),
        vm((S, 128), f32),
        vm((S, 128), f32),
        vm((NREG, NB, OROWS, D), bf16),
        vm((9, 8, D), f32),
        vm((2, 8, 128), f32),
        pltpu.SMEM((4,), jnp.int32),
        pltpu.SemaphoreType.DMA((1,)),
    ]
    out = pl.pallas_call(
        _kernel,
        out_shape=jax.ShapeDtypeStruct((NREG, NB, OROWS, D), bf16),
        in_specs=[pl.BlockSpec(memory_space=pl.ANY)] * len(args),
        out_specs=pl.BlockSpec(memory_space=pl.ANY),
        scratch_shapes=scratch,
        compiler_params=pltpu.CompilerParams(vmem_limit_bytes=100 * 1024 * 1024),
        name="adaln_h3_mod",
    )(*args)
    return out.reshape(1, S, D)
```
